```python
import os as _os
_os.environ.setdefault('JAX_PLATFORMS', 'cpu')
import jax
import jax.numpy as jnp

def _softmax(x, axis=-1):
    return jax.nn.softmax(x, axis=axis)

def _gelu(x):
    return jax.nn.gelu(x, approximate=True)

def _silu(x):
    return jax.nn.silu(x)

def _sigmoid(x):
    return jax.nn.sigmoid(x)

def _layernorm(x, axis=-1, eps=1e-05):
    m = jnp.mean(x, axis=axis, keepdims=True)
    v = jnp.var(x, axis=axis, keepdims=True)
    return (x - m) / jnp.sqrt(v + eps)

def _scatter_add(tgt, idx, src, axis=0):
    return tgt.at[idx].add(src)

def _segment_sum(src, seg, n):
    return jax.ops.segment_sum(src, seg, n)

class _Rng:

    def __init__(self, key):
        self._k = key

    def _next(self):
        self._k, sub = jax.random.split(self._k)
        return sub

    def normal(self, shape):
        return jax.random.normal(self._next(), shape, dtype=jnp.bfloat16)

    def randint(self, lo, hi, shape):
        return jax.random.randint(self._next(), shape, lo, hi, dtype=jnp.int32)

    def uniform(self, shape, lo=0.0, hi=1.0):
        return jax.random.uniform(self._next(), shape, jnp.bfloat16, lo, hi)

    def permutation(self, n):
        return jax.random.permutation(self._next(), n)
kernel_name = 'adaLN_cond__sliding_local_dilated__glu_gated_swiglu__prompt'

def setup_inputs():
    _rng = _Rng(jax.random.key(int.from_bytes(__import__("os").urandom(4), "little")))
    _w = lambda a: (lambda t: t.astype(jnp.bfloat16) if jnp.issubdtype(t.dtype, jnp.floating) else t)(jnp.asarray(a))

    def _A_setup():
        B, S, D = (1, 2048, 576)
        return {'x': _w((lambda *s: _rng.normal(s) * 0.05)(B, S, D)), 'wqkv': _w((lambda *s: _rng.normal(s) * 0.05)(D, 3 * D)), 'wo': _w((lambda *s: _rng.normal(s) * 0.05)(D, D))}
    _A_in = _A_setup()

    def _B_setup():
        B, S, D, F = (1, 2048, 576, 4608)
        return {'x': _w((lambda *s: _rng.normal(s) * 0.05)(B, S, D)), 'w1': _w((lambda *s: _rng.normal(s) * 0.8)(D, F) * (2.0 / D) ** 0.5), 'w3': _w((lambda *s: _rng.normal(s) * 0.8)(D, F) * (2.0 / D) ** 0.5), 'w2': _w((lambda *s: _rng.normal(s) * 0.8)(F, D) * (2.0 / F) ** 0.5)}
    _B_in = _B_setup()
    return {'A_x': _A_in['x'], 'A_wqkv': _A_in['wqkv'], 'A_wo': _A_in['wo'], 'B_x': _B_in['x'], 'B_w1': _B_in['w1'], 'B_w3': _B_in['w3'], 'B_w2': _B_in['w2'], 'c': _w((lambda *s: _rng.normal(s) * 0.05)(1, 576) * 8.0), 'w_mod': _w((lambda *s: _rng.normal(s) * 0.05)(576, 6 * 576) * 576 ** (-0.5) * 8.0)}

def reference(A_x, A_wqkv, A_wo, B_x, B_w1, B_w3, B_w2, c, w_mod):

    def _A_ref(x, wqkv, wo):
        B, S, D = x.shape
        H = 32
        Dh = D // H
        W, dil = (8, 2)
        qkv = (lambda x, *d: x.transpose(*d))((x @ wqkv).reshape(B, S, 3, H, Dh), 2, 0, 3, 1, 4)
        q, k, v = (qkv[0], qkv[1], qkv[2])
        scale = Dh ** (-0.5)
        pos = jnp.arange(S)
        off = jnp.arange(W) * dil
        idx = pos[:, None] - off[None, :]
        mask = idx >= 0
        idx_c = jnp.where(mask, idx, 0).reshape(-1)
        kg = k[:, :, idx_c, :].reshape(B, H, S, W, Dh)
        vg = v[:, :, idx_c, :].reshape(B, H, S, W, Dh)
        logits = jnp.einsum('bhsd,bhswd->bhsw', q, kg) * scale
        logits = jnp.where(mask[None, None, :, :], logits, -1000000000.0)
        attn = _softmax(logits, axis=-1)
        o = jnp.einsum('bhsw,bhswd->bhsd', attn, vg)
        return (lambda x, *d: x.transpose(*d))(o, 0, 2, 1, 3).reshape(B, S, D) @ wo

    def _B_ref(x, w1, w3, w2):
        gate = jnp.einsum('bsd,df->bsf', x, w1)
        up = jnp.einsum('bsd,df->bsf', x, w3)
        h = _silu(gate) * up
        out = jnp.einsum('bsf,fd->bsd', h, w2)
        return out
    x = A_x
    mod = (_silu(c) @ w_mod).reshape(c.shape[0], 6, 1, -1)
    sa, ca, ga, sb, cb, gb = (mod[:, 0].copy(), mod[:, 1].copy(), mod[:, 2].copy(), mod[:, 3].copy(), mod[:, 4].copy(), mod[:, 5].copy())
    h = _layernorm(x, axis=-1) * (1 + ca) + sa
    x = x + ga * _A_ref(h, A_wqkv, A_wo)
    h = _layernorm(x, axis=-1) * (1 + cb) + sb
    x = x + gb * _B_ref(h, B_w1, B_w3, B_w2)
    return x
```

```python
import functools
import jax
import jax.numpy as jnp
import jax.experimental.pallas as pl
import jax.experimental.pallas.tpu as pltpu

S, D, F = 2048, 576, 4608
H, DH, W, DIL = 32, 18, 8, 2
HALO = 16
EPS = 1e-5
NT = (((1,), (1,)), ((), ()))
f32, bf16 = jnp.float32, jnp.bfloat16
LOG2E = 1.4426950408889634
HD = D // 2
HS = S // 2


def _ln_T(xT):
    m = jnp.sum(xT, axis=0, keepdims=True) * (1.0 / D)
    xc = xT - m
    v = jnp.sum(xc * xc, axis=0, keepdims=True) * (1.0 / D)
    return xc * jax.lax.rsqrt(v + EPS)


def wsum(a, b):
    return (a.astype(f32) + b.astype(f32)).astype(bf16)


def wdiff(a, b):
    return (a.astype(f32) - b.astype(f32)).astype(bf16)


def mm(a, b):
    return jnp.dot(a, b, preferred_element_type=f32)


def mmt(a, b):
    return jax.lax.dot_general(a, b, NT, preferred_element_type=f32)


def swiglu(g, u):
    t = 0.5 * g
    tu = t * u
    return tu + tu * jnp.tanh(t)


def make(TA=1024, RB=256, FC=512, R=16, ORDER=0):
    NA = S // TA
    NB = TA // RB
    NC = F // FC
    HC = FC // 2
    HB = RB // 2

    def kern(xT_ref, c_ref, wqkv_hbm, wo_hbm, w1_hbm, w3_hbm, w2T_hbm, wmod_hbm, out_ref,
             wqkv_v, wo_v, wmod_v, w1_v, w3_v, w2T_v, tq_s, wT_s, woT_s, mod_s, gcol_s,
             q_s, kv_s, o_s, x1_s, a_s, ht_s, acc_s, sems):
        i = pl.program_id(0)

        def cp(src, dst, k):
            return pltpu.make_async_copy(src, dst, sems.at[k])

        c_wqkv = cp(wqkv_hbm, wqkv_v, 0)
        c_wmod = cp(wmod_hbm, wmod_v, 1)
        c_wo = cp(wo_hbm, wo_v, 2)
        c_ffn = [cp(w1_hbm, w1_v, 3), cp(w3_hbm, w3_v, 4), cp(w2T_hbm, w2T_v, 5)]

        @pl.when(i == 0)
        @jax.named_scope("prologue")
        def _prologue():
            c_wqkv.start()
            c_wmod.start()
            c_wo.start()
            for d in c_ffn:
                d.start()
            c_wqkv.wait()
            for j in range(5):
                rows = 128 if j < 4 else 64
                blk = wqkv_v[j * 128:j * 128 + rows, :].astype(f32)
                tq_s[j, :, 0:rows] = blk.T
            for sec in range(3):
                for d in range(DH):
                    dst = sec * 512 + d * 32 if d < 16 else 1536 + sec * 64 + (d - 16) * 32
                    for j in range(5):
                        w = 128 if j < 4 else 64
                        g = tq_s[j, pl.ds(sec * D + d, H, stride=DH), :]
                        wT_s[dst:dst + 32, j * 128:j * 128 + w] = g[:, 0:w].astype(bf16)
            wT_s[1728:1792, :] = jnp.zeros((64, D), bf16)
            c_wmod.wait()
            cc = c_ref[...].astype(f32)
            sc = (cc * jax.nn.sigmoid(cc)).astype(bf16)
            mod = jnp.dot(jnp.broadcast_to(sc, (16, D)), wmod_v[...], preferred_element_type=f32)
            for m in range(6):
                mod_s[m] = mod[0:8, m * D:(m + 1) * D]
            for n, m in enumerate((2, 5)):
                row = mod[0:1, m * D:(m + 1) * D]
                gcol_s[n] = jnp.broadcast_to(row, (128, D)).T
            c_wo.wait()
            for j in range(5):
                w = 128 if j < 4 else 64
                tq_s[j, 0:D, 0:w] = wo_v[:, j * 128:j * 128 + w].astype(f32)
            for j in range(5):
                w = 128 if j < 4 else 64
                parts = [tq_s[j, pl.ds(d, H, stride=DH), :] for d in range(DH)]
                parts.append(jnp.zeros((64, 128), f32))
                p = jnp.concatenate(parts, axis=0)
                woT_s[j * 128:j * 128 + w, :] = p.T[0:w, :].astype(bf16)
            kv_s[:, TA:TA + HALO, :] = jnp.zeros((10, HALO, 128), f32)

        def s1(b):
            r = slice(b * RB, (b + 1) * RB)
            rk = slice(HALO + b * RB, HALO + (b + 1) * RB)
            xT = xT_ref[:, r].astype(f32)
            h1 = _ln_T(xT).T * (1.0 + mod_s[1, 0:1, :]) + mod_s[0, 0:1, :]
            qkv = mmt(h1.astype(bf16), wT_s[...])
            qscale = (DH ** -0.5) * LOG2E
            lane = jax.lax.broadcasted_iota(jnp.int32, (RB, 128), 1)
            for j in range(4):
                q_s[j, r, :] = qkv[:, j * 128:(j + 1) * 128] * qscale
                kv_s[j, rk, :] = qkv[:, 512 + j * 128:512 + (j + 1) * 128]
                kv_s[5 + j, rk, :] = qkv[:, 1024 + j * 128:1024 + (j + 1) * 128]
            t4 = qkv[:, 1536:1664]
            q_s[4, r, :] = jnp.where(lane < 64, t4 * qscale, 0.0)
            kv_s[4, rk, :] = pltpu.roll(t4, 64, 1)
            kv_s[9, rk, :] = qkv[:, 1664:1792]

        def s2(b):
            for r0 in range(b * RB, (b + 1) * RB, R):
                q = [q_s[j, r0:r0 + R, :] for j in range(5)]
                lg = []
                for w in range(W):
                    o0 = HALO + r0 - DIL * w
                    p = q[0] * kv_s[0, o0:o0 + R, :]
                    for j in range(1, 5):
                        p = p + q[j] * kv_s[j, o0:o0 + R, :]
                    p = p + pltpu.roll(p, 64, 1)
                    p = p + pltpu.roll(p, 32, 1)
                    if r0 < HALO and w > 0:
                        pos = i * TA + r0 + jax.lax.broadcasted_iota(jnp.int32, (R, 128), 0)
                        p = jnp.where(pos >= DIL * w, p, -1e9 * LOG2E)
                    lg.append(p)
                m = lg[0]
                for w in range(1, W):
                    m = jnp.maximum(m, lg[w])
                e = [jnp.exp2(l - m) for l in lg]
                den = e[0]
                for w in range(1, W):
                    den = den + e[w]
                inv = 1.0 / den
                for j in range(5):
                    a = e[0] * kv_s[5 + j, HALO + r0:HALO + r0 + R, :]
                    for w in range(1, W):
                        o0 = HALO + r0 - DIL * w
                        a = a + e[w] * kv_s[5 + j, o0:o0 + R, :]
                    o_s[r0:r0 + R, j * 128:(j + 1) * 128] = (a * inv).astype(bf16)

        def s3(b):
            r = slice(b * RB, (b + 1) * RB)
            attT = mmt(woT_s[...], o_s[r, :])
            ga = jnp.concatenate([gcol_s[0]] * (RB // 128), axis=1)
            x1T = xT_ref[:, r].astype(f32) + ga * attT
            col = pl.multiple_of(i * TA + b * RB, RB)
            x1_s[:, pl.ds(col, RB)] = x1T
            h = _ln_T(x1T).T * (1.0 + mod_s[4, 0:1, :]) + mod_s[3, 0:1, :]
            A11, A12, A21, A22 = h[:HB, 0:256], h[:HB, 256:512], h[HB:, 0:256], h[HB:, 256:512]
            rr = pl.ds(pl.multiple_of(i * (TA // 2) + b * HB, HB), HB)
            a_s[0, rr, :] = (A11 + A22).astype(bf16)
            a_s[1, rr, :] = (A21 + A22).astype(bf16)
            a_s[2, rr, :] = A11.astype(bf16)
            a_s[3, rr, :] = A22.astype(bf16)
            a_s[4, rr, :] = (A11 + A12).astype(bf16)
            a_s[5, rr, :] = (A21 - A11).astype(bf16)
            a_s[6, rr, :] = (A12 - A22).astype(bf16)
            ht_s[0, rr, :] = h[:HB, 512:576].astype(bf16)
            ht_s[1, rr, :] = h[HB:, 512:576].astype(bf16)
            acc_s[:, :, rr] = jnp.zeros((7, HD, HB), f32)

        @pl.when(i < NA)
        @jax.named_scope("phaseA")
        def _phase_a():
            kv_s[:, 0:HALO, :] = kv_s[:, TA:TA + HALO, :]
            if ORDER == 0:
                s1(0)
                for b in range(1, NB):
                    s1(b)
                    s2(b - 1)
                    s3(b - 1)
                s2(NB - 1)
                s3(NB - 1)
            elif ORDER == 1:
                for b in range(NB):
                    s1(b)
                for b in range(NB):
                    s2(b)
                    s3(b)
            elif ORDER == 2:
                for t in range(NB + 2):
                    if 0 <= t - 2 < NB:
                        s3(t - 2)
                    if t < NB:
                        s1(t)
                    if 0 <= t - 1 < NB:
                        s2(t - 1)

        @pl.when(i == NA)
        def _():
            for d in c_ffn:
                d.wait()

        @pl.when(i >= NA)
        @jax.named_scope("phaseB")
        def _phase_b():
            base = pl.multiple_of((i - NA) * FC, FC)
            n1 = pl.ds(base, HC)
            n2 = pl.ds(base + HC, HC)
            n = pl.ds(base, FC)

            def proj(w_ref):
                B11, B12, B21, B22 = w_ref[0:256, n1], w_ref[0:256, n2], w_ref[256:512, n1], w_ref[256:512, n2]
                wt = w_ref[512:576, n]
                T1 = mm(ht_s[0], wt)
                T2 = mm(ht_s[1], wt)
                M1 = mm(a_s[0], wsum(B11, B22))
                M2 = mm(a_s[1], B11)
                M3 = mm(a_s[2], wdiff(B12, B22))
                M4 = mm(a_s[3], wdiff(B21, B11))
                M5 = mm(a_s[4], B22)
                M6 = mm(a_s[5], wsum(B11, B12))
                M7 = mm(a_s[6], wsum(B21, B22))
                C11 = M1 + M4 - M5 + M7 + T1[:, :HC]
                C12 = M3 + M5 + T1[:, HC:]
                C21 = M2 + M4 + T2[:, :HC]
                C22 = M1 - M2 + M3 + M6 + T2[:, HC:]
                return C11, C12, C21, C22

            g = proj(w1_v)
            u = proj(w3_v)
            B11, B21, B12, B22 = [swiglu(gg, uu) for gg, uu in zip(g, u)]
            A11, A12, A21, A22 = w2T_v[0:HD, n1], w2T_v[0:HD, n2], w2T_v[HD:D, n1], w2T_v[HD:D, n2]
            acc_s[0] += mmt(wsum(A11, A22), (B11 + B22).astype(bf16))
            acc_s[1] += mmt(wsum(A21, A22), B11.astype(bf16))
            acc_s[2] += mmt(A11, (B12 - B22).astype(bf16))
            acc_s[3] += mmt(A22, (B21 - B11).astype(bf16))
            acc_s[4] += mmt(wsum(A11, A12), B22.astype(bf16))
            acc_s[5] += mmt(wdiff(A21, A11), (B11 + B12).astype(bf16))
            acc_s[6] += mmt(wdiff(A12, A22), (B21 + B22).astype(bf16))

        @pl.when(i == NA + NC - 1)
        @jax.named_scope("epilogue")
        def _epilogue():
            for t in range(HS // 128):
                blk, j = divmod(t * 128, HB)
                c1 = slice(blk * RB + j, blk * RB + j + 128)
                c2 = slice(blk * RB + HB + j, blk * RB + HB + j + 128)
                M1, M2, M3, M4, M5, M6, M7 = [acc_s[k, :, t * 128:(t + 1) * 128] for k in range(7)]
                g1, g2 = gcol_s[1, 0:HD, :], gcol_s[1, HD:D, :]
                out_ref[0:HD, c1] = (x1_s[0:HD, c1] + g1 * (M1 + M4 - M5 + M7)).astype(bf16)
                out_ref[0:HD, c2] = (x1_s[0:HD, c2] + g1 * (M3 + M5)).astype(bf16)
                out_ref[HD:D, c1] = (x1_s[HD:D, c1] + g2 * (M2 + M4)).astype(bf16)
                out_ref[HD:D, c2] = (x1_s[HD:D, c2] + g2 * (M1 - M2 + M3 + M6)).astype(bf16)

    def fn(A_x, A_wqkv, A_wo, B_x, B_w1, B_w3, B_w2, c, w_mod):
        xT = A_x[0].T
        w2T = B_w2.T
        hbm = pl.BlockSpec(memory_space=pl.ANY)
        outT = pl.pallas_call(
            kern,
            grid=(NA + NC,),
            in_specs=[pl.BlockSpec((D, TA), lambda i: (0, jnp.minimum(i, NA - 1))),
                      pl.BlockSpec((1, D), lambda i: (0, 0)),
                      hbm, hbm, hbm, hbm, hbm, hbm],
            out_specs=pl.BlockSpec((D, S), lambda i: (0, 0)),
            out_shape=jax.ShapeDtypeStruct((D, S), bf16),
            scratch_shapes=[
                pltpu.VMEM((D, 3 * D), bf16),
                pltpu.VMEM((D, D), bf16),
                pltpu.VMEM((D, 6 * D), bf16),
                pltpu.VMEM((D, F), bf16),
                pltpu.VMEM((D, F), bf16),
                pltpu.VMEM((D, F), bf16),
                pltpu.VMEM((5, 3 * D, 128), f32),
                pltpu.VMEM((1792, D), bf16),
                pltpu.VMEM((D, 640), bf16),
                pltpu.VMEM((6, 8, D), f32),
                pltpu.VMEM((2, D, 128), f32),
                pltpu.VMEM((5, TA, 128), f32),
                pltpu.VMEM((10, TA + HALO, 128), f32),
                pltpu.VMEM((TA, 640), bf16),
                pltpu.VMEM((D, S), f32),
                pltpu.VMEM((7, HS, 256), bf16),
                pltpu.VMEM((2, HS, 64), bf16),
                pltpu.VMEM((7, HD, HS), f32),
                pltpu.SemaphoreType.DMA((6,)),
            ],
            compiler_params=pltpu.CompilerParams(dimension_semantics=("arbitrary",),
                                                 vmem_limit_bytes=110 * 1024 * 1024),
            name="adaln_blk",
        )(xT, c, A_wqkv, A_wo, B_w1, B_w3, w2T, w_mod)
        return outT.T[None]

    return fn


_impl = make(TA=1024)


@jax.jit
def pallas_adaLN_cond__sliding_local_dilated__glu_gated_swiglu__prompt_kernel(
    A_x: jax.Array,
    A_wqkv: jax.Array,
    A_wo: jax.Array,
    B_x: jax.Array,
    B_w1: jax.Array,
    B_w3: jax.Array,
    B_w2: jax.Array,
    c: jax.Array,
    w_mod: jax.Array,
):
    return _impl(A_x, A_wqkv, A_wo, B_x, B_w1, B_w3, B_w2, c, w_mod)
```

```python
import functools
import numpy as np
import jax
import jax.numpy as jnp
import jax.experimental.pallas as pl
import jax.experimental.pallas.tpu as pltpu

S, D, F = 2048, 576, 4608
H, DH, W, DIL = 32, 18, 8, 2
HALO = 16
EPS = 1e-5
NT = (((1,), (1,)), ((), ()))
f32, bf16 = jnp.float32, jnp.bfloat16
LOG2E = 1.4426950408889634
HD = D // 2
HS = S // 2
RB = 256
HB = RB // 2
NBLK = S // RB
NQ = 1792


def _ln_T(xT):
    m = jnp.sum(xT, axis=0, keepdims=True) * (1.0 / D)
    xc = xT - m
    v = jnp.sum(xc * xc, axis=0, keepdims=True) * (1.0 / D)
    return xc * jax.lax.rsqrt(v + EPS)


def _ln_T1(xT):
    m = jnp.sum(xT, axis=0, keepdims=True) * (1.0 / D)
    m2 = jnp.sum(xT * xT, axis=0, keepdims=True) * (1.0 / D)
    v = jnp.maximum(m2 - m * m, 0.0)
    return (xT - m) * jax.lax.rsqrt(v + EPS)


def wsum(a, b):
    return (a.astype(f32) + b.astype(f32)).astype(bf16)


def wdiff(a, b):
    return (a.astype(f32) - b.astype(f32)).astype(bf16)


def mm(a, b):
    return jnp.dot(a, b, preferred_element_type=f32)


def mmt(a, b):
    return jax.lax.dot_general(a, b, NT, preferred_element_type=f32)


def swiglu(g, u):
    t = 0.5 * g
    tu = t * u
    return tu + tu * jnp.tanh(t)


def quads(x):
    m, n = x.shape[0] // 2, x.shape[1] // 2
    return [x[:m, :n], x[:m, n:], x[m:, :n], x[m:, n:]]


def lhs7(X):
    a, b, c, d = X
    return [a + d, c + d, a, d, a + b, c - a, b - d]


def rhs7(X):
    a, b, c, d = X
    return [a + d, a, b - d, c - a, d, a + b, c + d]


def rhs7n(X):
    a, b, c, d = X
    return [a + d, a, d - b, c - a, -d, a + b, c + d]


def out4(M):
    M1, M2, M3, M4, M5, M6, M7 = M
    return [(M1 + M7) + (M4 - M5), M3 + M5, M2 + M4, (M1 + M6) + (M3 - M2)]


def lin(terms):
    v = None
    for t, sg in terms:
        v = t if v is None else (v + t if sg > 0 else v - t)
    return v


INNER = [2, 4, 1, 3, 0, 5, 6]
OUTER = [2, 4, 3, 1, 0, 6, 5]
FIN = {4: 1, 1: 2, 6: 0, 5: 3}
RIDE = {2: (1, 1), 4: (1, 3), 3: (2, 1), 1: (2, 3), 0: (0, 1), 6: (0, 3), 5: (3, 3)}
PRE = {2: [(1, 0), (1, 2)], 3: [(2, 0), (2, 2)], 0: [(0, 0), (0, 2)], 6: [(3, 0), (3, 1)], 5: [(3, 2)]}
RT = [[(0, 1), (3, 1)], [(0, 1)], [(1, 1), (3, -1)], [(2, 1), (0, -1)], [(3, 1)], [(0, 1), (1, 1)], [(2, 1), (3, 1)]]
OQ = [2, 0, 3, 1]
DIN = [4, 1, 0, 5, 2, 3, 6]
QD = D // 4
QS = S // 4
QB = RB // 4


def _plan(DS):
    it = lambda a: [(a, b) for b in DIN]
    if DS == 2:
        return {11: it(4), 19: it(1) + it(0), 27: it(2) + it(5) + it(3) + it(6)}
    if DS == 3:
        return {11: it(4), 19: it(1), 25: it(2), 27: it(0) + it(5) + it(3) + it(6)}
    if DS == 4:
        return {11: it(4), 19: it(1) + it(0), 25: it(2), 27: it(5) + it(3) + it(6)}


def _after(const, x):
    cb = int(np.float32(const).view(np.int32))
    xi = jax.lax.bitcast_convert_type(x, jnp.int32)
    zi = jnp.maximum(jnp.minimum(xi, 0), cb)
    return jax.lax.bitcast_convert_type(zi, f32)


def _pk(x):
    return pltpu.bitcast(x, jnp.uint32)


def _up(x):
    return pltpu.bitcast(x, bf16)


def _ds(start, size, align):
    if isinstance(start, int):
        return pl.ds(start, size)
    return pl.ds(pl.multiple_of(start, align), size)


def make(FC=512, R=8, CH=0, SK=0, NG=4, ORD='312', TH=0, TN=14, SCOPES=True, DS=2, STR=0, SKH=1, SKT=0, ER=16, QP=8, KP=24, LN1P=1, APX=1):
    NC = F // FC
    HC = FC // 2
    scope = jax.named_scope if SCOPES else (lambda n: (lambda f: f))

    def kern(xT_hbm, c_ref, wqkv_hbm, wo_hbm, w1_hbm, w3_hbm, w2T_hbm, wmod_hbm, out_hbm,
             x_v, wqkv_v, wo_v, wmod_v, w1_v, w3_v, w2T_v, tq_s, wT_s, woT_s, mod_s, gcol_s,
             q_s, kv_s, o_s, x1_s, a_s, ht_s, acc_s, out_v, sems, osems):

        def cp(src, dst, k):
            return pltpu.make_async_copy(src, dst, sems.at[k])

        c_x0 = cp(xT_hbm.at[:, 0:2 * RB], x_v.at[:, 0:2 * RB], 0)
        c_ma = cp(wmod_hbm.at[:, 0:2 * D], wmod_v.at[:, 0:2 * D], 1)
        c_wq = [cp(wqkv_hbm.at[j * 128:min((j + 1) * 128, D), :], wqkv_v.at[j * 128:min((j + 1) * 128, D), :], 2 + j)
                for j in range(5)]
        c_wo = cp(wo_hbm, wo_v, 7)
        c_mb = cp(wmod_hbm.at[:, 2 * D:], wmod_v.at[:, 2 * D:], 8)
        c_x1 = cp(xT_hbm.at[:, 2 * RB:], x_v.at[:, 2 * RB:], 9)
        c_ffn = [cp(w1_hbm, w1_v, 10), cp(w3_hbm, w3_v, 11), cp(w2T_hbm, w2T_v, 12)]
        for d in [c_x0, c_ma] + c_wq + [c_wo, c_mb, c_x1] + c_ffn:
            d.start()

        def silu_c():
            cc = c_ref[...].astype(f32)
            return jnp.broadcast_to((cc * jax.nn.sigmoid(cc)).astype(bf16), (16, D))

        def s1(r0, par):
            r = _ds(r0, RB, RB)
            rk = pl.ds(HALO, RB)
            if not (isinstance(r0, int) and r0 == 0):
                kv_s[par, :, 0:HALO, :] = kv_s[1 - par, :, RB:RB + HALO, :]
            xT = x_v[:, r].astype(f32)
            h1 = ((_ln_T1 if LN1P else _ln_T)(xT).T * (1.0 + mod_s[1, 0:1, :]) + mod_s[0, 0:1, :]).astype(bf16)
            wT = jnp.concatenate([_up(wT_s[j]) for j in range(4)] + [_up(wT_s[4])[:, 0:64]], axis=1)
            qkv = mmt(h1, wT)
            lane = jax.lax.broadcasted_iota(jnp.int32, (RB, 128), 1)
            for j in range(4):
                q_s[par, j, 0:RB, :] = qkv[:, j * 128:(j + 1) * 128]
                kv_s[par, j, rk, :] = qkv[:, 512 + j * 128:512 + (j + 1) * 128]
                kv_s[par, 5 + j, rk, :] = qkv[:, 1024 + j * 128:1024 + (j + 1) * 128]
            t4 = qkv[:, 1536:1664]
            q_s[par, 4, 0:RB, :] = jnp.where(lane < 64, t4, 0.0)
            kv_s[par, 4, rk, :] = pltpu.roll(t4, 64, 1)
            kv_s[par, 9, rk, :] = qkv[:, 1664:1792]
            return qkv

        def s2(par, first=False, tsrc=None, SK=SK):
            qscale = (DH ** -0.5) * LOG2E
            ngrp = RB // R
            st = {}
            qv = q_s.at[par]
            kvv = kv_s.at[par]
            ov = o_s.at[par]

            def rows(g, off):
                if STR:
                    return pl.ds((g // 2) * 16 + (g % 2) + off, R, stride=2)
                return pl.ds(g * R + off, R)

            def stage_a(g):
                q = [qv[j, rows(g, 0), :] * qscale for j in range(5)]
                ps = []
                for w in range(W):
                    rw = rows(g, HALO - DIL * w)
                    p = q[0] * kvv[0, rw, :]
                    for j in range(1, 5):
                        p = p + q[j] * kvv[j, rw, :]
                    ps.append(p)
                P = jnp.concatenate(ps, axis=0)
                st[g] = (P, pltpu.roll(P, 64, 1))

            def stage_b(g):
                P, Pr = st[g]
                P = P + Pr
                st[g] = (P, pltpu.roll(P, 32, 1))

            def stage_c(g):
                P, Pr = st.pop(g)
                P = P + Pr
                lg = [P[w * R:(w + 1) * R] for w in range(W)]
                if first and g < 2:
                    it = jax.lax.broadcasted_iota(jnp.int32, (R, 128), 0)
                    pos = (g + 2 * it) if STR else (g * R + it)
                    lg = [lg[0]] + [jnp.where(pos >= DIL * w, lg[w], -1e9 * LOG2E) for w in range(1, W)]
                m = jnp.maximum(jnp.maximum(jnp.maximum(lg[0], lg[1]), jnp.maximum(lg[2], lg[3])),
                                jnp.maximum(jnp.maximum(lg[4], lg[5]), jnp.maximum(lg[6], lg[7])))
                e = [jnp.exp2(l - m) for l in lg]
                den = ((e[0] + e[1]) + (e[2] + e[3])) + ((e[4] + e[5]) + (e[6] + e[7]))
                inv = pl.reciprocal(den, approx=True) if APX else 1.0 / den
                for j in range(5):
                    a = e[0] * kvv[5 + j, rows(g, HALO), :]
                    for w in range(1, W):
                        a = a + e[w] * kvv[5 + j, rows(g, HALO - DIL * w), :]
                    if g % 2 == 0:
                        st[('o', j)] = a * inv
                    elif STR:
                        ov[j, (g // 2) * 8:(g // 2) * 8 + 8, :] = pltpu.pack_elementwise(
                            [st.pop(('o', j)), a * inv], packed_dtype=bf16).astype(jnp.uint32)
                    else:
                        both = jnp.concatenate([st.pop(('o', j)), a * inv], axis=0)
                        ov[j, (g // 2) * 8:(g // 2) * 8 + 8, :] = _pk(both.astype(bf16))

            for i in range(ngrp + 2 * SK):
                if i < ngrp:
                    stage_a(i)
                if 0 <= i - SK < ngrp:
                    stage_b(i - SK)
                if 0 <= i - 2 * SK < ngrp:
                    stage_c(i - 2 * SK)

        def s3(r0, par):
            r = _ds(r0, RB, RB)
            o = jnp.concatenate([_up(o_s[par, j]) for j in range(5)], axis=1)
            woT = jnp.concatenate([_up(woT_s[j]) for j in range(5)], axis=1)
            attT = mmt(woT, o)
            ga = jnp.concatenate([gcol_s[0]] * (RB // 128), axis=1)
            x1T = x_v[:, r].astype(f32) + ga * attT
            x1_s[:, r] = x1T
            h = (_ln_T1 if LN1P else _ln_T)(x1T).T * (1.0 + mod_s[4, 0:1, :]) + mod_s[3, 0:1, :]
            rr = _ds(r0 // 8, QB // 2, QB // 2)
            for ka, y in enumerate(lhs7(quads(h[:, 0:512]))):
                for kb, z in enumerate(lhs7(quads(y))):
                    a_s[ka * 7 + kb, rr, :] = _pk(z.astype(bf16))
            for i in range(4):
                ht_s[i, rr, :] = _pk(h[i * QB:(i + 1) * QB, 512:576].astype(bf16))

        @scope("prologue")
        def _prologue():
            kv_s[0, :, 0:HALO, :] = jnp.zeros((10, HALO, 128), f32)
            wT_s[:, 3 * D // 2:NQ // 2, :] = jnp.zeros((5, (NQ - 3 * D) // 2, 128), jnp.uint32)
            tq_s[4] = jnp.zeros((3 * D, 128), f32)
            def zero(k, carry):
                acc_s[k // 7, pl.ds((k % 7) * 7, 7)] = jnp.zeros((7, QD, 128), f32)
                return carry
            jax.lax.fori_loop(0, 28, zero, 0)
            c_x0.wait()
            c_ma.wait()
            mod = mm(silu_c(), wmod_v[:, 0:2 * D])
            for m in range(2):
                mod_s[m] = mod[0:8, m * D:(m + 1) * D]
            for j in range(5):
                w = 128 if j < 4 else 64
                c_wq[j].wait()
                tq_s[j, :, 0:w] = wqkv_v[j * 128:j * 128 + w, :].astype(f32).T
                for sec in range(3):
                    for d in range(DH):
                        dst = sec * 512 + d * 32 if d < 16 else 1536 + sec * 64 + (d - 16) * 32
                        g = tq_s[j, pl.ds(sec * D + d, H, stride=DH), :]
                        wT_s[j, dst // 2:dst // 2 + 16, :] = _pk(g.astype(bf16))
        _prologue()

        @scope("head0")
        def _head0():
            s1(0, 0)
        _head0()

        @scope("head1")
        def _head1():
            c_wo.wait()
            c_mb.wait()
            mod = mm(silu_c(), wmod_v[:, 2 * D:])
            for m in (3, 4):
                mod_s[m] = mod[0:8, (m - 2) * D:(m - 1) * D]
            for n, m in enumerate((2, 5)):
                row = mod[0:1, (m - 2) * D:(m - 1) * D]
                gcol_s[n] = jnp.broadcast_to(row, (128, D)).T
            for j in range(5):
                w = 128 if j < 4 else 64
                tq_s[j, 0:D, 0:w] = wo_v[:, j * 128:j * 128 + w].astype(f32)
            for j in range(5):
                w = 128 if j < 4 else 64
                parts = [tq_s[j, pl.ds(d, H, stride=DH), 0:w] for d in range(DH)] if False else \
                        [tq_s[j, pl.ds(d, H, stride=DH), :] for d in range(DH)]
                parts.append(jnp.zeros((64, 128), f32))
                pT = jnp.concatenate(parts, axis=0).T[0:w, :].astype(bf16)
                for k in range(5):
                    woT_s[k, j * 64:j * 64 + w // 2, :] = _pk(pT[:, k * 128:(k + 1) * 128])
            s2(0, first=True, SK=SKH)
            s1(RB, 1)
            c_x1.wait()
        _head1()

        @scope("steady")
        def _steady():
            def step(t, par):
                r0 = t * RB
                toks = [None]
                for k in ORD:
                    if k == '3':
                        s3(r0 - 2 * RB, par)
                    elif k == '2':
                        s2(1 - par, tsrc=toks[0] if TH else None)
                    else:
                        toks[0] = s1(r0, par)

            def body(t, carry):
                for par in range(2):
                    pl.when(t % 2 == par)(functools.partial(step, t, par))
                return carry
            jax.lax.fori_loop(2, NBLK, body, 0)
        _steady()

        @scope("tail")
        def _tail():
            s3(S - 2 * RB, 0)
            s2(1, SK=SKT)
            s3(S - RB, 1)
            for d in c_ffn:
                d.wait()
        _tail()

        outs = [pltpu.make_async_copy(out_v.at[:, t * QS:(t + 1) * QS], out_hbm.at[:, t * QS:(t + 1) * QS],
                                      osems.at[t]) for t in range(4)]

        def finish(t):
            cs = slice(t * QS, (t + 1) * QS)
            for r0 in range(0, QD, ER):
                Mo = [out4([acc_s[t, a * 7 + b, r0:r0 + ER, :] for b in range(7)]) for a in range(7)]
                Cq = [out4([Mo[a][i] for a in range(7)]) for i in range(4)]
                for mo in range(2):
                    for mi in range(2):
                        rs = slice(mo * HD + mi * QD + r0, mo * HD + mi * QD + r0 + ER)
                        row = jnp.concatenate([Cq[mi * 2 + nn][mo * 2 + 1 - hh] for nn in range(2) for hh in range(2)],
                                              axis=1)
                        gcol = jnp.concatenate([gcol_s[1, rs, :]] * 4, axis=1)
                        out_v[rs, cs] = (x1_s[rs, cs] + gcol * row).astype(bf16)

        @scope("phaseB")
        def _phase_b():
            def body(ci, carry):
                n = pl.ds(pl.multiple_of(ci * FC, FC), FC)
                ws = (w1_v, w3_v)
                W1 = [rhs7(quads(w[0:512, n].astype(f32))) for w in ws]
                wt = [w[512:576, n] for w in ws]
                A1 = lhs7(quads(w2T_v[:, n].astype(f32)))
                T, Mo, Cb, Pp = [{}, {}], [[None] * 7, [None] * 7], [{}, {}], [{}, {}]
                Hb, cache, wave = {}, {}, [0]
                plan = _plan(DS)

                def tail(x, oq, iq):
                    i = (oq // 2) * 2 + iq // 2
                    j = (oq % 2) * 2 + iq % 2
                    return mm(_up(ht_s[i]), wt[x][:, j * 128:(j + 1) * 128])

                def hblk(oq, j):
                    kk, nn = divmod(j, 2)
                    if (oq, j) not in cache:
                        parts = []
                        for t in range(4):
                            rs = slice((2 * t + nn) * QB, (2 * t + nn + 1) * QB)
                            parts += [Hb[(oq, kk)][rs], Hb[(oq, 2 + kk)][rs]]
                        cache[(oq, j)] = jnp.concatenate(parts, axis=0)
                    return cache[(oq, j)]

                def ditem(a, b):
                    if a not in cache:
                        cache[a] = lhs7(quads(A1[a]))
                    terms = [(hblk(OQ[i], j), s1 * s2) for i, s1 in RT[a] for j, s2 in RT[b]]
                    if len(terms) == 4:
                        terms = [terms[0], terms[3], terms[1], terms[2]]
                    r = mmt(cache[a][b].astype(bf16), lin(terms).astype(bf16))
                    for t in range(4):
                        acc_s[t, a * 7 + b] += r[:, t * 128:(t + 1) * 128]

                def after_wave():
                    for da, db in plan.get(wave[0], []):
                        ditem(da, db)
                    wave[0] += 1

                def chain(x, v, terms, iq):
                    for k, sg in terms:
                        if iq == 1:
                            sg = -sg
                        v = v + Mo[x][k][iq] if sg > 0 else v - Mo[x][k][iq]
                    return v

                def final(x, a, iq):
                    if a == 0:
                        m1 = Mo[x][0][iq] if iq != 1 else -Mo[x][0][iq]
                        Pp[x][(0, iq)] = chain(x, m1, [(3, 1), (4, -1)], iq)
                        Pp[x][(3, iq)] = chain(x, m1, [(2, 1), (1, -1)], iq)
                    if a not in FIN:
                        return
                    oq = FIN[a]
                    t = T[x][(oq, iq)]
                    if oq in (0, 3):
                        v = chain(x, t, [(a, 1)], iq) + Pp[x][(oq, iq)]
                    else:
                        v = chain(x, t, {1: [(4, 1), (2, 1)], 2: [(1, 1), (3, 1)]}[oq], iq)
                    Cb[x][(oq, iq)] = v
                    if x == 1:
                        Hb[(oq, iq)] = swiglu(Cb[0][(oq, iq)], v)

                for a in OUTER:
                    for x in range(2):
                        for key in PRE.get(a, []):
                            T[x][key] = tail(x, *key)
                    for x in range(2):
                        B2 = [b.astype(bf16) for b in rhs7n(quads(W1[x][a]))]
                        M = [None] * 7
                        for b in INNER[:4]:
                            M[b] = mm(_up(a_s[a * 7 + b]), B2[b])
                        SA = [M[3] + M[4], M[2] + M[4], M[1] + M[3], M[2] + M[1]]
                        Mo[x][a] = [None, SA[1], SA[2], None]
                        final(x, a, 1)
                        final(x, a, 2)
                        after_wave()
                        for b in INNER[4:]:
                            M[b] = mm(_up(a_s[a * 7 + b]), B2[b])
                        T[x][RIDE[a]] = tail(x, *RIDE[a])
                        Mo[x][a] = [(M[0] + M[6]) + SA[0], SA[1], SA[2], (M[0] + M[5]) - SA[3]]
                        final(x, a, 0)
                        final(x, a, 3)
                        after_wave()
                return carry
            jax.lax.fori_loop(0, NC, body, 0)
        _phase_b()

        @scope("epilogue")
        def _epilogue():
            for t in range(4):
                finish(t)
                outs[t].start()
            for t in range(4):
                outs[t].wait()
        _epilogue()

    def fn(A_x, A_wqkv, A_wo, B_x, B_w1, B_w3, B_w2, c, w_mod):
        xT = A_x[0].T
        w2T = B_w2.T
        hbm = pl.BlockSpec(memory_space=pl.ANY)
        outT = pl.pallas_call(
            kern,
            in_specs=[hbm, pl.BlockSpec((1, D), lambda: (0, 0)), hbm, hbm, hbm, hbm, hbm, hbm],
            out_specs=hbm,
            out_shape=jax.ShapeDtypeStruct((D, S), bf16),
            scratch_shapes=[
                pltpu.VMEM((D, S), bf16),
                pltpu.VMEM((D, 3 * D), bf16),
                pltpu.VMEM((D, D), bf16),
                pltpu.VMEM((D, 6 * D), bf16),
                pltpu.VMEM((D, F), bf16),
                pltpu.VMEM((D, F), bf16),
                pltpu.VMEM((D, F), bf16),
                pltpu.VMEM((5, 3 * D, 128), f32),
                pltpu.VMEM((5, NQ // 2, 128), jnp.uint32),
                pltpu.VMEM((5, D // 2, 128), jnp.uint32),
                pltpu.VMEM((6, 8, D), f32),
                pltpu.VMEM((2, D, 128), f32),
                pltpu.VMEM((2, 5, RB + QP, 128), f32),
                pltpu.VMEM((2, 10, RB + HALO + KP, 128), f32),
                pltpu.VMEM((2, 5, HB, 128), jnp.uint32),
                pltpu.VMEM((D, S), f32),
                pltpu.VMEM((49, QS // 2, 128), jnp.uint32),
                pltpu.VMEM((4, QS // 2, 64), jnp.uint32),
                pltpu.VMEM((4, 49, QD, 128), f32),
                pltpu.VMEM((D, S), bf16),
                pltpu.SemaphoreType.DMA((13,)),
                pltpu.SemaphoreType.DMA((4,)),
            ],
            compiler_params=pltpu.CompilerParams(vmem_limit_bytes=110 * 1024 * 1024),
            name="adaln_blk",
        )(xT, c, A_wqkv, A_wo, B_w1, B_w3, w2T, w_mod)
        return outT.T[None]

    return fn


_impl = make(SCOPES=False)


@jax.jit
def pallas_adaLN_cond__sliding_local_dilated__glu_gated_swiglu__prompt_kernel(
    A_x: jax.Array,
    A_wqkv: jax.Array,
    A_wo: jax.Array,
    B_x: jax.Array,
    B_w1: jax.Array,
    B_w3: jax.Array,
    B_w2: jax.Array,
    c: jax.Array,
    w_mod: jax.Array,
):
    return _impl(A_x, A_wqkv, A_wo, B_x, B_w1, B_w3, B_w2, c, w_mod)
```

```python
import functools
import numpy as np
import jax
import jax.numpy as jnp
import jax.experimental.pallas as pl
import jax.experimental.pallas.tpu as pltpu

S, D, F = 2048, 576, 4608
H, DH, W, DIL = 32, 18, 8, 2
HALO = 16
EPS = 1e-5
NT = (((1,), (1,)), ((), ()))
f32, bf16 = jnp.float32, jnp.bfloat16
LOG2E = 1.4426950408889634
HD = D // 2
HS = S // 2
RB = 256
HB = RB // 2
NBLK = S // RB
NQ = 1792


def _ln_T(xT):
    m = jnp.sum(xT, axis=0, keepdims=True) * (1.0 / D)
    xc = xT - m
    v = jnp.sum(xc * xc, axis=0, keepdims=True) * (1.0 / D)
    return xc * jax.lax.rsqrt(v + EPS)


def _ln_T1(xT):
    m = jnp.sum(xT, axis=0, keepdims=True) * (1.0 / D)
    m2 = jnp.sum(xT * xT, axis=0, keepdims=True) * (1.0 / D)
    v = jnp.maximum(m2 - m * m, 0.0)
    return (xT - m) * jax.lax.rsqrt(v + EPS)


def wsum(a, b):
    return (a.astype(f32) + b.astype(f32)).astype(bf16)


def wdiff(a, b):
    return (a.astype(f32) - b.astype(f32)).astype(bf16)


def mm(a, b):
    return jnp.dot(a, b, preferred_element_type=f32)


def mmt(a, b):
    return jax.lax.dot_general(a, b, NT, preferred_element_type=f32)


def swiglu(g, u):
    t = 0.5 * g
    tu = t * u
    return tu + tu * jnp.tanh(t)


def quads(x):
    m, n = x.shape[0] // 2, x.shape[1] // 2
    return [x[:m, :n], x[:m, n:], x[m:, :n], x[m:, n:]]


def lhs7(X):
    a, b, c, d = X
    return [a + d, c + d, a, d, a + b, c - a, b - d]


def rhs7(X):
    a, b, c, d = X
    return [a + d, a, b - d, c - a, d, a + b, c + d]


def rhs7n(X):
    a, b, c, d = X
    return [a + d, a, d - b, c - a, -d, a + b, c + d]


def out4(M):
    M1, M2, M3, M4, M5, M6, M7 = M
    return [(M1 + M7) + (M4 - M5), M3 + M5, M2 + M4, (M1 + M6) + (M3 - M2)]


def lin(terms):
    v = None
    for t, sg in terms:
        v = t if v is None else (v + t if sg > 0 else v - t)
    return v


INNER = [2, 4, 1, 3, 0, 5, 6]
OUTER = [2, 4, 3, 1, 0, 6, 5]
FIN = {4: 1, 1: 2, 6: 0, 5: 3}
RIDE = {2: (1, 1), 4: (1, 3), 3: (2, 1), 1: (2, 3), 0: (0, 1), 6: (0, 3), 5: (3, 3)}
PRE = {2: [(1, 0), (1, 2)], 3: [(2, 0), (2, 2)], 0: [(0, 0), (0, 2)], 6: [(3, 0), (3, 1)], 5: [(3, 2)]}
RT = [[(0, 1), (3, 1)], [(0, 1)], [(1, 1), (3, -1)], [(2, 1), (0, -1)], [(3, 1)], [(0, 1), (1, 1)], [(2, 1), (3, 1)]]
OQ = [2, 0, 3, 1]
DIN = [4, 1, 0, 5, 2, 3, 6]
QD = D // 4
QS = S // 4
QB = RB // 4


def _plan(DS):
    it = lambda a: [(a, b) for b in DIN]
    if isinstance(DS, dict):
        return {w: sum([it(a) for a in v], []) for w, v in DS.items()}
    if DS == 7:
        z = lambda p, q: [y for pair in zip(it(p), it(q)) for y in pair]
        return {19: it(0), 27: z(2, 4) + it(5) + z(3, 1) + it(6)}
    if DS == 2:
        return {11: it(4), 19: it(1) + it(0), 27: it(2) + it(5) + it(3) + it(6)}
    if DS == 3:
        return {11: it(4), 19: it(1), 25: it(2), 27: it(0) + it(5) + it(3) + it(6)}
    if DS == 5:
        return {11: it(4), 17: [(0, -1)], 19: it(1) + it(0), 24: [(2, -1)], 25: [(5, -1)],
                27: it(2) + [(3, -1)] + it(5) + [(6, -1)] + it(3) + it(6)}
    if DS == 6:
        return {11: it(4), 17: [(0, -1)], 19: it(1), 24: [(2, -1)], 25: [(5, -1)],
                27: it(0) + [(3, -1)] + it(2) + [(6, -1)] + it(5) + it(3) + it(6)}
    if DS == 4:
        return {11: it(4), 19: it(1) + it(0), 25: it(2), 27: it(5) + it(3) + it(6)}


def _sched(NH, DS):
    it = lambda hf, a: [('d', hf, a, b) for b in DIN]
    seq = []
    if NH == 1:
        plan = _plan(DS)
        for w in range(28):
            seq.append(('g', 0, w))
            seq += [('d', 0, a, b) for a, b in plan.get(w, [])]
        return seq
    if DS == 10:
        seq += [('g', 0, w) for w in range(28)]
        pend = sum([it(0, a) for a in (4, 1, 0, 2, 5, 3, 6)], [])
        own = {}
        for w in range(28):
            seq.append(('g', 1, w))
            seq += pend[:2]
            pend = pend[2:]
            if w == 24:
                seq += [('e', 0), ('e', 1)]
        seq += sum([it(1, a) for a in (4, 1, 0, 2, 5, 3, 6)], [])
    elif DS == 11:
        for w in range(28):
            seq.append(('g', 0, w))
            if w == 19:
                seq += it(0, 4) + it(0, 1)
        pend = sum([it(0, a) for a in (0, 2, 5, 3, 6)], [])
        for w in range(28):
            seq.append(('g', 1, w))
            seq += pend[:4]
            pend = pend[4:]
            if w == 9:
                seq += [('e', 0)]
            if w == 16:
                seq += [('e', 1)]
            if w == 19:
                seq += it(1, 4) + it(1, 1) + it(1, 0)[:1]
        seq += it(1, 0)[1:] + sum([it(1, a) for a in (2, 5, 3, 6)], [])
    elif DS == 12:
        for w in range(28):
            seq.append(('g', 0, w))
            if w == 19:
                seq += it(0, 4) + it(0, 1)
        for w in range(28):
            seq.append(('g', 1, w))
            if w == 3:
                seq += it(0, 0) + it(0, 2)
            if w == 9:
                seq += it(0, 5) + it(0, 3)
            if w == 11:
                seq += it(0, 6) + it(1, 4)
                seq += [('e', 0)]
            if w == 17:
                seq += [('e', 1)]
            if w == 19:
                seq += it(1, 1) + it(1, 0)
        seq += sum([it(1, a) for a in (2, 5, 3, 6)], [])
    return seq


def _after(const, x):
    cb = int(np.float32(const).view(np.int32))
    xi = jax.lax.bitcast_convert_type(x, jnp.int32)
    zi = jnp.maximum(jnp.minimum(xi, 0), cb)
    return jax.lax.bitcast_convert_type(zi, f32)


def _pk(x):
    return pltpu.bitcast(x, jnp.uint32)


def _up(x):
    return pltpu.bitcast(x, bf16)


def _ds(start, size, align):
    if isinstance(start, int):
        return pl.ds(start, size)
    return pl.ds(pl.multiple_of(start, align), size)


def make(FC=512, R=8, CH=0, SK=0, NG=4, ORD='312', TH=0, TN=14, SCOPES=True, DS=2, DBG=0, HS2=0, HG=12, HN=1024, EM=1, ECH=(16, 32, 48, 48), KS=1, KO=0, MERGE=0, Z0=14, Z1=23, NP0=1, NOZ=0, OV=2, DI=(4, 0, 1, 5, 2, 3, 6), PLAN=None, NH=1, INL=0, HF=(), CK=16, STR=0, SKH=1, SKT=0, ER=16, QP=8, KP=24, LN1P=1, APX=1):
    NC = F // FC
    global OUTER, FIN, RIDE, PRE, DIN
    if OV == 0:
        OUTER = [2, 4, 3, 1, 0, 6, 5]
        FIN = {4: 1, 1: 2, 6: 0, 5: 3}
        RIDE = {2: (1, 1), 4: (1, 3), 3: (2, 1), 1: (2, 3), 0: (0, 1), 6: (0, 3), 5: (3, 3)}
        PRE = {2: [(1, 0), (1, 2)], 3: [(2, 0), (2, 2)], 0: [(0, 0), (0, 2)], 6: [(3, 0), (3, 1)], 5: [(3, 2)]}
    elif OV == 1:
        OUTER = [4, 2, 1, 3, 0, 6, 5]
        FIN = {2: 1, 3: 2, 6: 0, 5: 3}
        RIDE = {4: (1, 1), 2: (1, 3), 1: (2, 1), 3: (2, 3), 0: (0, 1), 6: (0, 3), 5: (3, 3)}
        PRE = {4: [(1, 0), (1, 2)], 1: [(2, 0), (2, 2)], 0: [(0, 0), (0, 2)], 6: [(3, 0), (3, 1)], 5: [(3, 2)]}
    elif OV == 2:
        OUTER = [4, 2, 1, 3, 0, 6, 5]
        FIN = {2: 1, 3: 2, 6: 0, 5: 3}
        RIDE = {4: (1, 1), 2: (1, 3), 1: (2, 1), 3: (2, 3), 0: (0, 1), 6: (0, 3), 5: (3, 3)}
        PRE = {4: [(3, 2)], 2: [(1, 0), (1, 2)], 3: [(2, 0), (2, 2)], 6: [(0, 0), (0, 2)], 5: [(3, 0), (3, 1)]}
    if DI is not None:
        DIN = list(DI)
    HC = FC // 2
    scope = jax.named_scope if SCOPES else (lambda n: (lambda f: f))

    def kern(xT_hbm, c_hbm, wqkv_hbm, wo_hbm, w1_hbm, w3_hbm, w2T_hbm, wmod_hbm, out_hbm,
             x_v, wqkv_v, wo_v, wmod_v, w1_v, w3_v, w2T_v, tq_s, wT_s, woT_s, mod_s, gcol_s,
             q_s, kv_s, o_s, x1_s, a_s, acc_s, out_v, part_s, c_ref, sems, xsems, osems):

        a_b, o_b, wT_b, woT_b = [r.bitcast(bf16) for r in (a_s, o_s, wT_s, woT_s)]

        def cp(src, dst, k):
            return pltpu.make_async_copy(src, dst, sems.at[k])

        def c_x(t):
            cols = _ds(t * RB, RB, RB)
            return pltpu.make_async_copy(xT_hbm.at[:, cols], x_v.at[:, cols], xsems.at[t])

        MB = 23 * 128
        c_ma = cp(wmod_hbm.at[:, 0:2 * D], wmod_v.at[:, 0:2 * D], 1)
        c_wq = [cp(wqkv_hbm.at[j * 128:min((j + 1) * 128, D), :], wqkv_v.at[j * 128:min((j + 1) * 128, D), :], 2 + j)
                for j in range(5)]
        c_wo = cp(wo_hbm, wo_v, 7)
        c_mb = cp(wmod_hbm.at[:, 2 * D:MB], wmod_v.at[:, 2 * D:MB], 8)
        c_mc = cp(wmod_hbm.at[:, MB:], wmod_v.at[:, MB:], 9)
        c_ffn = [cp(w1_hbm, w1_v, 10), cp(w3_hbm, w3_v, 11), cp(w2T_hbm, w2T_v, 12)]
        c_c = cp(c_hbm, c_ref, 0)
        for k, d in enumerate([c_x(0), c_wq[0], c_c, c_ma] + c_wq[1:] + [c_wo, c_x(1), c_mb]
                              + [c_x(t) for t in range(2, NBLK)] + [c_mc] + c_ffn):
            d.start(priority=0 if k < NP0 else 1)

        def WT(d, name):
            if DBG:
                with jax.named_scope(name):
                    d.wait()
            else:
                d.wait()

        def silu_c():
            cc = c_ref[...].astype(f32)
            return jnp.broadcast_to((cc * jax.nn.sigmoid(cc)).astype(bf16), (16, D))

        def modulate1(xn):
            return (xn * (1.0 + mod_s[1, 0:1, :]) + mod_s[0, 0:1, :]).astype(bf16)

        def wT(js):
            js = list(js)
            return wT_b[:, js[0] * 128:min((js[-1] + 1) * 128, D)]

        def store_qkv(qkv, par):
            rk = pl.ds(HALO, RB)
            lane = jax.lax.broadcasted_iota(jnp.int32, (RB, 128), 1)
            for j in range(4):
                q_s[par, j, 0:RB, :] = qkv[:, j * 128:(j + 1) * 128]
                kv_s[par, j, rk, :] = qkv[:, 512 + j * 128:512 + (j + 1) * 128]
                kv_s[par, 5 + j, rk, :] = qkv[:, 1024 + j * 128:1024 + (j + 1) * 128]
            t4 = qkv[:, 1536:1664]
            q_s[par, 4, 0:RB, :] = jnp.where(lane < 64, t4, 0.0)
            kv_s[par, 4, rk, :] = pltpu.roll(t4, 64, 1)
            kv_s[par, 9, rk, :] = qkv[:, 1664:1792]

        def s1(r0, par):
            kv_s[par, :, 0:HALO, :] = kv_s[1 - par, :, RB:RB + HALO, :]
            xT = x_v[:, _ds(r0, RB, RB)].astype(f32)
            h1 = modulate1(_ln_T1(xT).T)
            if KS == 0:
                qkv = mmt(h1, wT(range(5)))
            elif KS == 1:
                tl = mmt(h1[:, 512:576], wT([4]))
                qkv = mmt(h1[:, 0:512], wT(range(4))) + tl
            elif KS == 2:
                mn = mmt(h1[:, 0:512], wT(range(4)))
                qkv = mn + mmt(h1[:, 512:576], wT([4]))
            elif KS == 3:
                cols = []
                for n0 in range(0, NQ, 512):
                    n1 = min(n0 + 512, NQ)
                    tl = mmt(h1[:, 512:576], wT([4])[n0:n1])
                    cols.append(mmt(h1[:, 0:512], wT(range(4))[n0:n1]) + tl)
                qkv = jnp.concatenate(cols, axis=1)
            store_qkv(qkv, par)

        def s2(par, first=False, tsrc=None, SK=SK, glo=0, ghi=None):
            qscale = (DH ** -0.5) * LOG2E
            ngrp = RB // R
            st = {}
            qv = q_s.at[par]
            kvv = kv_s.at[par]

            def rows(g, off):
                if STR:
                    return pl.ds((g // 2) * 16 + (g % 2) + off, R, stride=2)
                return pl.ds(g * R + off, R)

            def stage_a(g):
                q = [qv[j, rows(g, 0), :] * qscale for j in range(5)]
                ps = []
                for w in range(W):
                    rw = rows(g, HALO - DIL * w)
                    p = q[0] * kvv[0, rw, :]
                    for j in range(1, 5):
                        p = p + q[j] * kvv[j, rw, :]
                    ps.append(p)
                P = jnp.concatenate(ps, axis=0)
                st[g] = (P, pltpu.roll(P, 64, 1))

            def stage_b(g):
                P, Pr = st[g]
                P = P + Pr
                st[g] = (P, pltpu.roll(P, 32, 1))

            def stage_c(g):
                P, Pr = st.pop(g)
                P = P + Pr
                lg = [P[w * R:(w + 1) * R] for w in range(W)]
                if first and g < 2:
                    it = jax.lax.broadcasted_iota(jnp.int32, (R, 128), 0)
                    pos = (g + 2 * it) if STR else (g * R + it)
                    lg = [lg[0]] + [jnp.where(pos >= DIL * w, lg[w], -1e9 * LOG2E) for w in range(1, W)]
                m = jnp.maximum(jnp.maximum(jnp.maximum(lg[0], lg[1]), jnp.maximum(lg[2], lg[3])),
                                jnp.maximum(jnp.maximum(lg[4], lg[5]), jnp.maximum(lg[6], lg[7])))
                e = [jnp.exp2(l - m) for l in lg]
                den = ((e[0] + e[1]) + (e[2] + e[3])) + ((e[4] + e[5]) + (e[6] + e[7]))
                inv = pl.reciprocal(den, approx=True) if APX else 1.0 / den
                for j in range(5):
                    a = e[0] * kvv[5 + j, rows(g, HALO), :]
                    for w in range(1, W):
                        a = a + e[w] * kvv[5 + j, rows(g, HALO - DIL * w), :]
                    if g % 2 == 0:
                        st[('o', j)] = a * inv
                    elif STR:
                        ov[j, (g // 2) * 8:(g // 2) * 8 + 8, :] = pltpu.pack_elementwise(
                            [st.pop(('o', j)), a * inv], packed_dtype=bf16).astype(jnp.uint32)
                    else:
                        both = jnp.concatenate([st.pop(('o', j)), a * inv], axis=0)
                        o_b[par, (g // 2) * 16:(g // 2) * 16 + 16, j * 128:(j + 1) * 128] = both.astype(bf16)

            ghi = ngrp if ghi is None else ghi
            for i in range(glo, ghi + 2 * SK):
                if i < ghi:
                    stage_a(i)
                if glo <= i - SK < ghi:
                    stage_b(i - SK)
                if glo <= i - 2 * SK < ghi:
                    stage_c(i - 2 * SK)

        def s3(r0, par):
            r = _ds(r0, RB, RB)
            o = o_b[par]
            woT = woT_b[...]
            if KO == 0:
                attT = mmt(woT, o)
            elif KO == 1:
                tl = mmt(woT[:, 512:640], o[:, 512:640])
                attT = mmt(woT[:, 0:512], o[:, 0:512]) + tl
            elif KO == 2:
                mn = mmt(woT[:, 0:512], o[:, 0:512])
                attT = mn + mmt(woT[:, 512:640], o[:, 512:640])
            elif KO == 3:
                tl = jnp.concatenate([mmt(woT[0:HD, 512:640], o[:, 512:640]), mmt(woT[HD:D, 512:640], o[:, 512:640])], axis=0)
                attT = mmt(woT[:, 0:512], o[:, 0:512]) + tl
            ga = jnp.concatenate([gcol_s[0]] * (RB // 128), axis=1)
            x1T = x_v[:, r].astype(f32) + ga * attT
            x1_s[:, r] = x1T
            h = (_ln_T1 if LN1P else _ln_T)(x1T).T * (1.0 + mod_s[4, 0:1, :]) + mod_s[3, 0:1, :]
            rr = _ds(r0 // 4, QB, QB)
            for ka, y in enumerate(lhs7(quads(h[:, 0:512]))):
                for kb, z in enumerate(lhs7(quads(y))):
                    a_b[rr, (ka * 7 + kb) * 128:(ka * 7 + kb + 1) * 128] = z.astype(bf16)
            for i in range(4):
                a_b[rr, (49 + i) * 128:(49 + i) * 128 + 64] = h[i * QB:(i + 1) * QB, 512:576].astype(bf16)

        def prep_wq(j):
            w = 128 if j < 4 else 64
            tq_s[j, :, 0:w] = wqkv_v[j * 128:j * 128 + w, :].astype(f32).T
            for sec in range(3):
                for d in range(DH):
                    dst = sec * 512 + d * 32 if d < 16 else 1536 + sec * 64 + (d - 16) * 32
                    g = tq_s[j, pl.ds(sec * D + d, H, stride=DH), :]
                    wT_b[dst:dst + 32, j * 128:j * 128 + w] = g[:, 0:w].astype(bf16)

        def col_bcast(row):
            return jnp.broadcast_to(row, (128, D)).T

        @scope("prologue")
        def _prologue():
            kv_s[0, :, 0:HALO, :] = jnp.zeros((10, HALO, 128), f32)
            wT_b[3 * D:NQ, :] = jnp.zeros((NQ - 3 * D, 640), bf16)
            if not NOZ:
                def zero(k, carry):
                    acc_s[k // 7, pl.ds((k % 7) * 7, 7)] = jnp.zeros((7, QD, 128), f32)
                    return carry
                jax.lax.fori_loop(0, Z0, zero, 0)
            WT(c_x(0), 'wx0')
            WT(c_wq[0], 'wq0')
            xn = _ln_T1(x_v[:, 0:RB].astype(f32)).T
            prep_wq(0)
            if not NOZ:
                jax.lax.fori_loop(Z0, Z1, zero, 0)
            c_c.wait()
            WT(c_ma, 'wma')
            mod = mm(silu_c(), wmod_v[:, 0:2 * D])
            for m in range(2):
                mod_s[m] = mod[0:8, m * D:(m + 1) * D]
            h1 = modulate1(xn)
            WT(c_wq[1], 'wq1')
            part_s[...] = mmt(h1[:, 0:128], wT([0]))
            prep_wq(1)
            WT(c_wq[2], 'wq2')
            part_s[...] += mmt(h1[:, 128:256], wT([1]))
            prep_wq(2)
            WT(c_wq[3], 'wq3')
            WT(c_wq[4], 'wq4')
            part = part_s[...] + mmt(h1[:, 256:384], wT([2]))
            prep_wq(3)
            prep_wq(4)
            store_qkv(part + mmt(h1[:, 384:576], wT([3, 4])), 0)
        _prologue()

        def modb():
            WT(c_mb, 'wmb')
            mod = mm(silu_c(), wmod_v[:, 2 * D:MB])
            gcol_s[0] = col_bcast(mod[0:1, 0:D])
            mod_s[3] = mod[0:8, D:2 * D]
            mod_s[4] = mod[0:8, 2 * D:3 * D]
            if not NOZ:
                acc_s[3, (Z1 - 21) * 7:49] = jnp.zeros(((28 - Z1) * 7, QD, 128), f32)

        @scope("head1")
        def _head1():
            WT(c_wo, 'wwo')
            WT(c_x(1), 'wx1')
            for j in range(5):
                w = 128 if j < 4 else 64
                tq_s[j, 0:D, 0:w] = wo_v[:, j * 128:j * 128 + w].astype(f32)
            for j in range(5):
                w = 128 if j < 4 else 64
                parts = [tq_s[j, pl.ds(d, H, stride=DH), :] for d in range(DH)]
                parts.append(jnp.zeros((64, 128), f32))
                pT = jnp.concatenate(parts, axis=0).T[0:w, :].astype(bf16)
                woT_b[j * 128:j * 128 + w, :] = pT
            if not HS2:
                s2(0, first=True, SK=SKH)
                s1(RB, 1)
                modb()
                return
            s2(0, first=True, SK=SKH, ghi=HG)
            kv_s[1, :, 0:HALO, :] = kv_s[0, :, RB:RB + HALO, :]
            h1 = modulate1(_ln_T1(x_v[:, RB:2 * RB].astype(f32)).T)
            part_s[:, 0:HN] = (mmt(h1[:, 512:576], wT_b[0:HN, 512:576]) + mmt(h1[:, 0:512], wT_b[0:HN, 0:512]))
            modb()
            rest = mmt(h1[:, 512:576], wT_b[HN:NQ, 512:576]) + mmt(h1[:, 0:512], wT_b[HN:NQ, 0:512])
            store_qkv(jnp.concatenate([part_s[:, 0:HN], rest], axis=1), 1)
            s2(0, SK=SKH, glo=HG)
        _head1()

        @scope("steady")
        def _steady():
            def step(t, par):
                r0 = t * RB
                toks = [None]
                for k in ORD:
                    if k == '3':
                        s3(r0 - 2 * RB, par)
                    elif k == '2':
                        s2(1 - par, tsrc=toks[0] if TH else None)
                    else:
                        s1(r0, par)

            def body(t, carry):
                c_x(t).wait()
                for par in range(2):
                    pl.when(t % 2 == par)(functools.partial(step, t, par))
                return carry

            def body2(u, carry):
                t = 2 * u
                c_x(t).wait()
                c_x(t + 1).wait()
                step(t, 0)
                step(t + 1, 1)
                return carry
            if MERGE:
                jax.lax.fori_loop(1, NBLK // 2, body2, 0)
            else:
                jax.lax.fori_loop(2, NBLK, body, 0)
        _steady()

        @scope("tail")
        def _tail():
            c_mc.wait()
            mod = mm(silu_c(), wmod_v[:, MB - 128:])
            gcol_s[1] = col_bcast(mod[0:1, 64:64 + D])
            s3(S - 2 * RB, 0)
            s2(1, SK=SKT)
            s3(S - RB, 1)
            for d in c_ffn:
                d.wait()
        _tail()

        outs = [pltpu.make_async_copy(out_v.at[:, t * QS:(t + 1) * QS], out_hbm.at[:, t * QS:(t + 1) * QS],
                                      osems.at[t]) for t in range(4)]

        def finish(t, ronly=None):
            cs = slice(t * QS, (t + 1) * QS)
            for r0 in (range(0, QD, ER) if ronly is None else [ronly]):
                Mo = [out4([acc_s[t, a * 7 + b, r0:r0 + ER, :] for b in range(7)]) for a in range(7)]
                Cq = [out4([Mo[a][i] for a in range(7)]) for i in range(4)]
                for mo in range(2):
                    for mi in range(2):
                        rs = slice(mo * HD + mi * QD + r0, mo * HD + mi * QD + r0 + ER)
                        row = jnp.concatenate([Cq[mi * 2 + nn][mo * 2 + 1 - hh] for nn in range(2) for hh in range(2)],
                                              axis=1)
                        gcol = jnp.concatenate([gcol_s[1, rs, :]] * 4, axis=1)
                        out_v[rs, cs] = (x1_s[rs, cs] + gcol * row).astype(bf16)

        @scope("phaseB")
        def _phase_b():
            def body(ci, carry):
                n = pl.ds(pl.multiple_of(ci * FC, FC), FC)
                ws = (w1_v, w3_v)
                W1 = [rhs7(quads(w[0:512, n].astype(f32))) for w in ws]
                wt = [w[512:576, n] for w in ws]
                A1 = lhs7(quads(w2T_v[:, n].astype(f32)))
                shared = {}

                def accum(t, k, v):
                    if NOZ:
                        acc_s[t, k] = jnp.where(ci > 0, acc_s[t, k], 0.0) + v
                    else:
                        acc_s[t, k] += v
                NTL = 4 // NH
                PR_ = QS // NH

                def part(hf):
                    T, Mo, Cb, Pp = [{}, {}], [[None] * 7, [None] * 7], [{}, {}], [{}, {}]
                    Hb, cache, st = {}, {}, {}
                    pr = slice(hf * PR_, (hf + 1) * PR_)

                    def tail(x, oq, iq):
                        i = (oq // 2) * 2 + iq // 2
                        j = (oq % 2) * 2 + iq % 2
                        return mm(a_b[pr, (49 + i) * 128:(49 + i) * 128 + 64], wt[x][:, j * 128:(j + 1) * 128])

                    def hblk(oq, j):
                        kk, nn = divmod(j, 2)
                        if (oq, j) not in cache:
                            parts = []
                            for t in range(NTL):
                                rs = slice((2 * t + nn) * QB, (2 * t + nn + 1) * QB)
                                parts += [Hb[(oq, kk)][rs], Hb[(oq, 2 + kk)][rs]]
                            cache[(oq, j)] = jnp.concatenate(parts, axis=0)
                        return cache[(oq, j)]

                    def prep(a):
                        if ('P', a) in cache:
                            return
                        outs7 = [[] for _ in range(7)]
                        for r0 in range(0, NTL * 128, CK):
                            l1 = [lin([(hblk(OQ[i], j)[r0:r0 + CK], sg) for i, sg in RT[a]]) for j in range(4)]
                            for b, z in enumerate(rhs7(l1)):
                                outs7[b].append(z.astype(bf16))
                        cache[('P', a)] = [jnp.concatenate(z, axis=0) for z in outs7]

                    def ditem(a, b):
                        if b < 0:
                            return prep(a)
                        if ('A', a) not in shared:
                            shared[('A', a)] = [z.astype(bf16) for z in lhs7(quads(A1[a]))]
                        if a in HF:
                            prep(a)
                            r = mmt(shared[('A', a)][b], cache[('P', a)][b])
                            for t in range(NTL):
                                accum(hf * NTL + t, a * 7 + b, r[:, t * 128:(t + 1) * 128])
                            return
                        terms = [(hblk(OQ[i], j), s1 * s2) for i, s1 in RT[a] for j, s2 in RT[b]]
                        if len(terms) == 4:
                            terms = [terms[0], terms[3], terms[1], terms[2]]
                        r = mmt(shared[('A', a)][b], lin(terms).astype(bf16))
                        for t in range(NTL):
                            accum(hf * NTL + t, a * 7 + b, r[:, t * 128:(t + 1) * 128])

                    def chain(x, v, terms, iq):
                        for k, sg in terms:
                            if iq == 1:
                                sg = -sg
                            v = v + Mo[x][k][iq] if sg > 0 else v - Mo[x][k][iq]
                        return v

                    def final(x, a, iq):
                        if a == 0:
                            m1 = Mo[x][0][iq] if iq != 1 else -Mo[x][0][iq]
                            Pp[x][(0, iq)] = chain(x, m1, [(3, 1), (4, -1)], iq)
                            Pp[x][(3, iq)] = chain(x, m1, [(2, 1), (1, -1)], iq)
                        if a not in FIN:
                            return
                        oq = FIN[a]
                        t = T[x][(oq, iq)]
                        if oq in (0, 3):
                            v = chain(x, t, [(a, 1)], iq) + Pp[x][(oq, iq)]
                        else:
                            v = chain(x, t, [(a, 1), ({4: 2, 2: 4, 1: 3, 3: 1}[a], 1)], iq)
                        Cb[x][(oq, iq)] = v
                        if x == 1:
                            Hb[(oq, iq)] = swiglu(Cb[0][(oq, iq)], v)

                    def gwave(w):
                        a, x, h2 = OUTER[w // 4], (w // 2) % 2, w % 2
                        if w % 4 == 0:
                            for xx in range(2):
                                for key in PRE.get(a, []):
                                    T[xx][key] = tail(xx, *key)
                        if ('B', x, a) not in shared:
                            shared[('B', x, a)] = [z.astype(bf16) for z in rhs7n(quads(W1[x][a]))]
                        B2 = shared[('B', x, a)]
                        if h2 == 0:
                            M = st['M'] = [None] * 7
                            for b in INNER[:4]:
                                M[b] = mm(a_b[pr, (a * 7 + b) * 128:(a * 7 + b + 1) * 128], B2[b])
                            SA = st['SA'] = [M[3] + M[4], M[2] + M[4], M[1] + M[3], M[2] + M[1]]
                            Mo[x][a] = [None, SA[1], SA[2], None]
                            final(x, a, 1)
                            final(x, a, 2)
                        else:
                            M, SA = st['M'], st['SA']
                            for b in INNER[4:]:
                                M[b] = mm(a_b[pr, (a * 7 + b) * 128:(a * 7 + b + 1) * 128], B2[b])
                            T[x][RIDE[a]] = tail(x, *RIDE[a])
                            Mo[x][a] = [(M[0] + M[6]) + SA[0], SA[1], SA[2], (M[0] + M[5]) - SA[3]]
                            final(x, a, 0)
                            final(x, a, 3)
                    return gwave, ditem

                parts_ = [part(hf) for hf in range(NH)]
                for op in _sched(NH, DS if PLAN is None else PLAN):
                    if op[0] == 'g':
                        parts_[op[1]][0](op[2])
                    elif op[0] == 'd':
                        parts_[op[1]][1](op[2], op[3])
                    elif INL:
                        finish(op[1])
                        pl.when(ci == NC - 1)(outs[op[1]].start)
                return carry
            jax.lax.fori_loop(0, NC, body, 0)
        _phase_b()

        @scope("epilogue")
        def _epilogue():
            if EM == 0:
                for t in range(4):
                    finish(t)
                    outs[t].start()
                for t in range(4):
                    outs[t].wait()
                return
            cps = []
            r0 = 0
            for ci_, rows in enumerate(ECH):
                for r in range(r0, r0 + rows, ER):
                    for t in range(4):
                        finish(t, r)
                for mq in range(4):
                    rs = slice(mq * QD + r0, mq * QD + r0 + rows)
                    d = pltpu.make_async_copy(out_v.at[rs, :], out_hbm.at[rs, :], osems.at[ci_ * 4 + mq])
                    d.start()
                    cps.append(d)
                r0 += rows
            for d in cps:
                d.wait()
        _epilogue()

    def fn(A_x, A_wqkv, A_wo, B_x, B_w1, B_w3, B_w2, c, w_mod):
        xT = A_x[0].T
        w2T = B_w2.T
        hbm = pl.BlockSpec(memory_space=pl.ANY)
        outT = pl.pallas_call(
            kern,
            in_specs=[hbm] * 8,
            out_specs=hbm,
            out_shape=jax.ShapeDtypeStruct((D, S), bf16),
            scratch_shapes=[
                pltpu.VMEM((D, S), bf16),
                pltpu.VMEM((D, 3 * D), bf16),
                pltpu.VMEM((D, D), bf16),
                pltpu.VMEM((D, 6 * D), bf16),
                pltpu.VMEM((D, F), bf16),
                pltpu.VMEM((D, F), bf16),
                pltpu.VMEM((D, F), bf16),
                pltpu.VMEM((5, 3 * D, 128), f32),
                pltpu.VMEM((NQ // 2, 640), jnp.uint32),
                pltpu.VMEM((D // 2, 640), jnp.uint32),
                pltpu.VMEM((6, 8, D), f32),
                pltpu.VMEM((2, D, 128), f32),
                pltpu.VMEM((2, 5, RB + QP, 128), f32),
                pltpu.VMEM((2, 10, RB + HALO + KP, 128), f32),
                pltpu.VMEM((2, HB, 640), jnp.uint32),
                pltpu.VMEM((D, S), f32),
                pltpu.VMEM((QS // 2, 53 * 128), jnp.uint32),
                pltpu.VMEM((4, 49, QD, 128), f32),
                pltpu.VMEM((D, S), bf16),
                pltpu.VMEM((RB, NQ), f32),
                pltpu.VMEM((1, D), bf16),
                pltpu.SemaphoreType.DMA((13,)),
                pltpu.SemaphoreType.DMA((NBLK,)),
                pltpu.SemaphoreType.DMA((4 * len(ECH),)),
            ],
            compiler_params=pltpu.CompilerParams(vmem_limit_bytes=110 * 1024 * 1024),
            name="adaln_blk",
        )(xT, c, A_wqkv, A_wo, B_w1, B_w3, w2T, w_mod)
        return outT.T[None]

    return fn


_impl = make(SCOPES=False)


@jax.jit
def pallas_adaLN_cond__sliding_local_dilated__glu_gated_swiglu__prompt_kernel(
    A_x: jax.Array,
    A_wqkv: jax.Array,
    A_wo: jax.Array,
    B_x: jax.Array,
    B_w1: jax.Array,
    B_w3: jax.Array,
    B_w2: jax.Array,
    c: jax.Array,
    w_mod: jax.Array,
):
    return _impl(A_x, A_wqkv, A_wo, B_x, B_w1, B_w3, B_w2, c, w_mod)
```

```python
import functools

import jax
import jax.numpy as jnp
import jax.experimental.pallas as pl
import jax.experimental.pallas.tpu as pltpu

S, D, F = 2048, 576, 4608
H, DH, W, DIL = 32, 18, 8, 2
EPS = 1e-5
LOG2E = 1.4426950408889634
f32, bf16, u32 = jnp.float32, jnp.bfloat16, jnp.uint32

HALO = 16
RB = 256
NBLK = S // RB
GR = 8
NQ = 1792
KM = 512
FC = 512
HD, QD, QS, QB = D // 2, D // 4, S // 4, RB // 4
MB = 23 * 128
ER = 16
ECH = (16, 32, 48, 48)
Z0, Z1 = 14, 23


def _mm(a, b):
    return jnp.dot(a, b, preferred_element_type=f32)


def _mmt(a, b):
    return jax.lax.dot_general(a, b, (((1,), (1,)), ((), ())), preferred_element_type=f32)


def _ln_t(xt):
    m = jnp.sum(xt, axis=0, keepdims=True) * (1.0 / D)
    m2 = jnp.sum(xt * xt, axis=0, keepdims=True) * (1.0 / D)
    v = jnp.maximum(m2 - m * m, 0.0)
    return (xt - m) * jax.lax.rsqrt(v + EPS)


def _swiglu(g, u):
    t = 0.5 * g
    tu = t * u
    return tu + tu * jnp.tanh(t)


def _ds(start, size):
    if isinstance(start, int):
        return pl.ds(start, size)
    return pl.ds(pl.multiple_of(start, size), size)


def _qkv_row(sec, d):
    return sec * 512 + d * 32 if d < 16 else 1536 + sec * 64 + (d - 16) * 32


def _quads(x):
    m, n = x.shape[0] // 2, x.shape[1] // 2
    return [x[:m, :n], x[:m, n:], x[m:, :n], x[m:, n:]]


def _lhs7(x):
    a, b, c, d = x
    return [a + d, c + d, a, d, a + b, c - a, b - d]


def _rhs7(x):
    a, b, c, d = x
    return [a + d, a, b - d, c - a, d, a + b, c + d]


def _rhs7n(x):
    a, b, c, d = x
    return [a + d, a, d - b, c - a, -d, a + b, c + d]


def _out4(m):
    m1, m2, m3, m4, m5, m6, m7 = m
    return [(m1 + m7) + (m4 - m5), m3 + m5, m2 + m4, (m1 + m6) + (m3 - m2)]


def _lin(terms):
    v = None
    for t, sg in terms:
        v = t if v is None else (v + t if sg > 0 else v - t)
    return v


RHS_TERMS = [[(0, 1), (3, 1)], [(0, 1)], [(1, 1), (3, -1)], [(2, 1), (0, -1)], [(3, 1)], [(0, 1), (1, 1)],
             [(2, 1), (3, 1)]]
INNER = [2, 4, 1, 3, 0, 5, 6]
OUTER = [4, 2, 1, 3, 0, 6, 5]
FIN = {2: (1, 4), 3: (2, 1), 6: (0, None), 5: (3, None)}
RIDE = {4: (1, 1), 2: (1, 3), 1: (2, 1), 3: (2, 3), 0: (0, 1), 6: (0, 3), 5: (3, 3)}
PRE = {4: [(3, 2)], 2: [(1, 0), (1, 2)], 3: [(2, 0), (2, 2)], 6: [(0, 0), (0, 2)], 5: [(3, 0), (3, 1)]}
DOWN_Q = [2, 0, 3, 1]
DOWN_IN = [4, 0, 1, 5, 2, 3, 6]
DOWN_AT = {11: [4], 19: [1, 0], 27: [2, 5, 3, 6]}


def _kernel(xt_hbm, c_hbm, wqkv_hbm, wo_hbm, w1_hbm, w3_hbm, w2t_hbm, wmod_hbm, out_hbm,
            x_v, c_v, wqkv_v, wo_v, wmod_v, w1_v, w3_v, w2t_v, tq_s, wt_s, wot_s, mod_s, gcol_s,
            part_s, q_s, kv_s, o_s, x1_s, a_s, acc_s, out_v, sems, xsems, osems):
    a_b, o_b, wt_b, wot_b = [r.bitcast(bf16) for r in (a_s, o_s, wt_s, wot_s)]

    def cp(src, dst, k):
        return pltpu.make_async_copy(src, dst, sems.at[k])

    def c_x(t):
        cols = _ds(t * RB, RB)
        return pltpu.make_async_copy(xt_hbm.at[:, cols], x_v.at[:, cols], xsems.at[t])

    c_c = cp(c_hbm, c_v, 0)
    c_ma = cp(wmod_hbm.at[:, 0:2 * D], wmod_v.at[:, 0:2 * D], 1)
    c_wq = [cp(wqkv_hbm.at[j * 128:min((j + 1) * 128, D), :], wqkv_v.at[j * 128:min((j + 1) * 128, D), :], 2 + j)
            for j in range(5)]
    c_wo = cp(wo_hbm, wo_v, 7)
    c_mb = cp(wmod_hbm.at[:, 2 * D:MB], wmod_v.at[:, 2 * D:MB], 8)
    c_mc = cp(wmod_hbm.at[:, MB:], wmod_v.at[:, MB:], 9)
    c_ffn = [cp(w1_hbm, w1_v, 10), cp(w3_hbm, w3_v, 11), cp(w2t_hbm, w2t_v, 12)]
    c_x(0).start(priority=0)
    for d in ([c_wq[0], c_c, c_ma] + c_wq[1:] + [c_wo, c_x(1), c_mb] + [c_x(t) for t in range(2, NBLK)]
              + [c_mc] + c_ffn):
        d.start(priority=1)

    def mod_cols(lo, hi):
        cc = c_v[...].astype(f32)
        sc = jnp.broadcast_to((cc * jax.nn.sigmoid(cc)).astype(bf16), (16, D))
        return _mm(sc, wmod_v[:, lo:hi])

    def col_bcast(row):
        return jnp.broadcast_to(row, (128, D)).T

    def modulate1(xn):
        return (xn * (1.0 + mod_s[1, 0:1, :]) + mod_s[0, 0:1, :]).astype(bf16)

    def store_qkv(qkv, par):
        rk = pl.ds(HALO, RB)
        lane = jax.lax.broadcasted_iota(jnp.int32, (RB, 128), 1)
        for j in range(4):
            q_s[par, j] = qkv[:, j * 128:(j + 1) * 128]
            kv_s[par, j, rk, :] = qkv[:, 512 + j * 128:512 + (j + 1) * 128]
            kv_s[par, 5 + j, rk, :] = qkv[:, 1024 + j * 128:1024 + (j + 1) * 128]
        t4 = qkv[:, 1536:1664]
        q_s[par, 4] = jnp.where(lane < 64, t4, 0.0)
        kv_s[par, 4, rk, :] = pltpu.roll(t4, 64, 1)
        kv_s[par, 9, rk, :] = qkv[:, 1664:1792]

    def s1(r0, par):
        kv_s[par, :, 0:HALO, :] = kv_s[1 - par, :, RB:RB + HALO, :]
        h1 = modulate1(_ln_t(x_v[:, _ds(r0, RB)].astype(f32)).T)
        tl = _mmt(h1[:, KM:D], wt_b[:, KM:D])
        store_qkv(_mmt(h1[:, 0:KM], wt_b[:, 0:KM]) + tl, par)

    def s2(par, first=False, skew=0):
        qscale = (DH ** -0.5) * LOG2E
        ngrp = RB // GR
        st = {}

        def kv(j, g, w):
            return kv_s[par, j, pl.ds(g * GR + HALO - DIL * w, GR), :]

        def scores(g):
            q = [q_s[par, j, g * GR:(g + 1) * GR, :] * qscale for j in range(5)]
            ps = []
            for w in range(W):
                p = q[0] * kv(0, g, w)
                for j in range(1, 5):
                    p = p + q[j] * kv(j, g, w)
                ps.append(p)
            p = jnp.concatenate(ps, axis=0)
            st[g] = (p, pltpu.roll(p, 64, 1))

        def fold(g):
            p, pr = st[g]
            p = p + pr
            st[g] = (p, pltpu.roll(p, 32, 1))

        def mix(g):
            p, pr = st.pop(g)
            p = p + pr
            lg = [p[w * GR:(w + 1) * GR] for w in range(W)]
            if first and g * GR < HALO:
                pos = g * GR + jax.lax.broadcasted_iota(jnp.int32, (GR, 128), 0)
                lg = [lg[0]] + [jnp.where(pos >= DIL * w, lg[w], -1e9 * LOG2E) for w in range(1, W)]
            m = jnp.maximum(jnp.maximum(jnp.maximum(lg[0], lg[1]), jnp.maximum(lg[2], lg[3])),
                            jnp.maximum(jnp.maximum(lg[4], lg[5]), jnp.maximum(lg[6], lg[7])))
            e = [jnp.exp2(l - m) for l in lg]
            den = ((e[0] + e[1]) + (e[2] + e[3])) + ((e[4] + e[5]) + (e[6] + e[7]))
            inv = pl.reciprocal(den, approx=True)
            inv = inv * (2.0 - den * inv)
            for j in range(5):
                a = e[0] * kv(5 + j, g, 0)
                for w in range(1, W):
                    a = a + e[w] * kv(5 + j, g, w)
                if g % 2 == 0:
                    st[('o', j)] = a * inv
                else:
                    both = jnp.concatenate([st.pop(('o', j)), a * inv], axis=0)
                    o_b[par, (g - 1) * GR:(g + 1) * GR, j * 128:(j + 1) * 128] = both.astype(bf16)

        for i in range(ngrp + 2 * skew):
            if i < ngrp:
                scores(i)
            if 0 <= i - skew < ngrp:
                fold(i - skew)
            if 0 <= i - 2 * skew < ngrp:
                mix(i - 2 * skew)

    def s3(r0, par):
        r = _ds(r0, RB)
        att = _mmt(wot_b[...], o_b[par])
        ga = jnp.concatenate([gcol_s[0]] * (RB // 128), axis=1)
        x1 = x_v[:, r].astype(f32) + ga * att
        x1_s[:, r] = x1
        h = _ln_t(x1).T * (1.0 + mod_s[3, 0:1, :]) + mod_s[2, 0:1, :]
        rr = _ds(r0 // 4, QB)
        for ka, y in enumerate(_lhs7(_quads(h[:, 0:KM]))):
            for kb, z in enumerate(_lhs7(_quads(y))):
                a_b[rr, (ka * 7 + kb) * 128:(ka * 7 + kb + 1) * 128] = z.astype(bf16)
        for i in range(4):
            a_b[rr, (49 + i) * 128:(49 + i) * 128 + 64] = h[i * QB:(i + 1) * QB, KM:D].astype(bf16)

    def prep_wq(j):
        w = 128 if j < 4 else 64
        tq_s[j, :, 0:w] = wqkv_v[j * 128:j * 128 + w, :].astype(f32).T
        for sec in range(3):
            for d in range(DH):
                g = tq_s[j, pl.ds(sec * D + d, H, stride=DH), :]
                dst = _qkv_row(sec, d)
                wt_b[dst:dst + 32, j * 128:j * 128 + w] = g[:, 0:w].astype(bf16)

    def prep_wo():
        for j in range(5):
            w = 128 if j < 4 else 64
            tq_s[j, 0:D, 0:w] = wo_v[:, j * 128:j * 128 + w].astype(f32)
        for j in range(5):
            w = 128 if j < 4 else 64
            parts = [tq_s[j, pl.ds(d, H, stride=DH), :] for d in range(DH)] + [jnp.zeros((64, 128), f32)]
            wot_b[j * 128:j * 128 + w, :] = jnp.concatenate(parts, axis=0).T[0:w, :].astype(bf16)

    def clear(k, carry):
        acc_s[k // 7, pl.ds((k % 7) * 7, 7)] = jnp.zeros((7, QD, 128), f32)
        return carry

    kv_s[0, :, 0:HALO, :] = jnp.zeros((10, HALO, 128), f32)
    wt_b[3 * D:NQ, :] = jnp.zeros((NQ - 3 * D, 640), bf16)
    tq_s[4] = jnp.zeros((3 * D, 128), f32)
    jax.lax.fori_loop(0, Z0, clear, 0)
    c_x(0).wait()
    c_wq[0].wait()
    xn = _ln_t(x_v[:, 0:RB].astype(f32)).T
    prep_wq(0)
    jax.lax.fori_loop(Z0, Z1, clear, 0)
    c_c.wait()
    c_ma.wait()
    mod = mod_cols(0, 2 * D)
    mod_s[0] = mod[0:8, 0:D]
    mod_s[1] = mod[0:8, D:2 * D]
    h1 = modulate1(xn)
    c_wq[1].wait()
    part_s[...] = _mmt(h1[:, 0:128], wt_b[:, 0:128])
    prep_wq(1)
    c_wq[2].wait()
    part_s[...] += _mmt(h1[:, 128:256], wt_b[:, 128:256])
    prep_wq(2)
    c_wq[3].wait()
    c_wq[4].wait()
    part = part_s[...] + _mmt(h1[:, 256:384], wt_b[:, 256:384])
    prep_wq(3)
    prep_wq(4)
    store_qkv(part + _mmt(h1[:, 384:D], wt_b[:, 384:D]), 0)

    c_wo.wait()
    c_x(1).wait()
    prep_wo()
    s2(0, first=True, skew=1)
    s1(RB, 1)
    c_mb.wait()
    mod = mod_cols(2 * D, MB)
    gcol_s[0] = col_bcast(mod[0:1, 0:D])
    mod_s[2] = mod[0:8, D:2 * D]
    mod_s[3] = mod[0:8, 2 * D:3 * D]
    acc_s[3, (Z1 - 21) * 7:49] = jnp.zeros(((28 - Z1) * 7, QD, 128), f32)

    def a_step(t, par):
        s3((t - 2) * RB, par)
        s1(t * RB, par)
        s2(1 - par)

    def a_body(t, carry):
        c_x(t).wait()
        for par in range(2):
            pl.when(t % 2 == par)(functools.partial(a_step, t, par))
        return carry

    jax.lax.fori_loop(2, NBLK, a_body, 0)

    c_mc.wait()
    gcol_s[1] = col_bcast(mod_cols(MB - 128, 6 * D)[0:1, 64:64 + D])
    s3(S - 2 * RB, 0)
    s2(1)
    s3(S - RB, 1)
    for d in c_ffn:
        d.wait()

    def b_body(ci, carry):
        n = _ds(ci * FC, FC)
        w_out = [_rhs7(_quads(w[0:KM, n].astype(f32))) for w in (w1_v, w3_v)]
        w_tail = [w[KM:D, n] for w in (w1_v, w3_v)]
        w2_out = _lhs7(_quads(w2t_v[:, n].astype(f32)))
        tails, mo, gate, psum = [{}, {}], [[None] * 7, [None] * 7], {}, [{}, {}]
        hid, hblk = {}, {}

        def tail(x, oq, iq):
            i, j = (oq // 2) * 2 + iq // 2, (oq % 2) * 2 + iq % 2
            return _mm(a_b[:, (49 + i) * 128:(49 + i) * 128 + 64], w_tail[x][:, j * 128:(j + 1) * 128])

        def chain(x, v, terms, iq):
            for k, sg in terms:
                v = v + mo[x][k][iq] if (sg > 0) != (iq == 1) else v - mo[x][k][iq]
            return v

        def final(x, a, iq):
            if a == 0:
                m1 = mo[x][0][iq] if iq != 1 else -mo[x][0][iq]
                psum[x][(0, iq)] = chain(x, m1, [(3, 1), (4, -1)], iq)
                psum[x][(3, iq)] = chain(x, m1, [(2, 1), (1, -1)], iq)
            if a not in FIN:
                return
            oq, partner = FIN[a]
            if partner is None:
                v = chain(x, tails[x][(oq, iq)], [(a, 1)], iq) + psum[x][(oq, iq)]
            else:
                v = chain(x, tails[x][(oq, iq)], [(a, 1), (partner, 1)], iq)
            if x == 0:
                gate[(oq, iq)] = v
            else:
                hid[(oq, iq)] = _swiglu(gate[(oq, iq)], v)

        def hidden(oq, j):
            if (oq, j) not in hblk:
                kk, nn = divmod(j, 2)
                parts = []
                for t in range(4):
                    rs = slice((2 * t + nn) * QB, (2 * t + nn + 1) * QB)
                    parts += [hid[(oq, kk)][rs], hid[(oq, 2 + kk)][rs]]
                hblk[(oq, j)] = jnp.concatenate(parts, axis=0)
            return hblk[(oq, j)]

        def down(wave):
            for a in DOWN_AT.get(wave, []):
                lhs = [z.astype(bf16) for z in _lhs7(_quads(w2_out[a]))]
                for b in DOWN_IN:
                    terms = [(hidden(DOWN_Q[i], j), si * sj) for i, si in RHS_TERMS[a] for j, sj in RHS_TERMS[b]]
                    if len(terms) == 4:
                        terms = [terms[0], terms[3], terms[1], terms[2]]
                    r = _mmt(lhs[b], _lin(terms).astype(bf16))
                    for t in range(4):
                        acc_s[t, a * 7 + b] += r[:, t * 128:(t + 1) * 128]

        wave = 0
        for a in OUTER:
            for x in range(2):
                for key in PRE.get(a, []):
                    tails[x][key] = tail(x, *key)
            for x in range(2):
                rhs = [z.astype(bf16) for z in _rhs7n(_quads(w_out[x][a]))]
                m = [None] * 7
                for b in INNER[:4]:
                    m[b] = _mm(a_b[:, (a * 7 + b) * 128:(a * 7 + b + 1) * 128], rhs[b])
                sa = [m[3] + m[4], m[2] + m[4], m[1] + m[3], m[2] + m[1]]
                mo[x][a] = [None, sa[1], sa[2], None]
                final(x, a, 1)
                final(x, a, 2)
                down(wave)
                for b in INNER[4:]:
                    m[b] = _mm(a_b[:, (a * 7 + b) * 128:(a * 7 + b + 1) * 128], rhs[b])
                tails[x][RIDE[a]] = tail(x, *RIDE[a])
                mo[x][a] = [(m[0] + m[6]) + sa[0], sa[1], sa[2], (m[0] + m[5]) - sa[3]]
                final(x, a, 0)
                final(x, a, 3)
                down(wave + 1)
                wave += 2
        return carry

    jax.lax.fori_loop(0, F // FC, b_body, 0)

    copies = []
    r0 = 0
    for ck, rows in enumerate(ECH):
        for r in range(r0, r0 + rows, ER):
            for t in range(4):
                cs = slice(t * QS, (t + 1) * QS)
                mo = [_out4([acc_s[t, a * 7 + b, r:r + ER, :] for b in range(7)]) for a in range(7)]
                cq = [_out4([mo[a][i] for a in range(7)]) for i in range(4)]
                for mq in range(4):
                    rs = slice(mq * QD + r, mq * QD + r + ER)
                    row = jnp.concatenate([cq[(mq % 2) * 2 + nn][(mq // 2) * 2 + 1 - hh]
                                           for nn in range(2) for hh in range(2)], axis=1)
                    gb = jnp.concatenate([gcol_s[1, rs, :]] * 4, axis=1)
                    out_v[rs, cs] = (x1_s[rs, cs] + gb * row).astype(bf16)
        for mq in range(4):
            rs = slice(mq * QD + r0, mq * QD + r0 + rows)
            d = pltpu.make_async_copy(out_v.at[rs, :], out_hbm.at[rs, :], osems.at[ck * 4 + mq])
            d.start()
            copies.append(d)
        r0 += rows
    for d in copies:
        d.wait()


@jax.jit
def pallas_adaLN_cond__sliding_local_dilated__glu_gated_swiglu__prompt_kernel(
    A_x: jax.Array,
    A_wqkv: jax.Array,
    A_wo: jax.Array,
    B_x: jax.Array,
    B_w1: jax.Array,
    B_w3: jax.Array,
    B_w2: jax.Array,
    c: jax.Array,
    w_mod: jax.Array,
):
    del B_x
    hbm = pl.BlockSpec(memory_space=pl.ANY)
    out_t = pl.pallas_call(
        _kernel,
        in_specs=[hbm] * 8,
        out_specs=hbm,
        out_shape=jax.ShapeDtypeStruct((D, S), bf16),
        scratch_shapes=[
            pltpu.VMEM((D, S), bf16),
            pltpu.VMEM((1, D), bf16),
            pltpu.VMEM((D, 3 * D), bf16),
            pltpu.VMEM((D, D), bf16),
            pltpu.VMEM((D, 6 * D), bf16),
            pltpu.VMEM((D, F), bf16),
            pltpu.VMEM((D, F), bf16),
            pltpu.VMEM((D, F), bf16),
            pltpu.VMEM((5, 3 * D, 128), f32),
            pltpu.VMEM((NQ // 2, 640), u32),
            pltpu.VMEM((D // 2, 640), u32),
            pltpu.VMEM((4, 8, D), f32),
            pltpu.VMEM((2, D, 128), f32),
            pltpu.VMEM((RB, NQ), f32),
            pltpu.VMEM((2, 5, RB, 128), f32),
            pltpu.VMEM((2, 10, RB + HALO, 128), f32),
            pltpu.VMEM((2, RB // 2, 640), u32),
            pltpu.VMEM((D, S), f32),
            pltpu.VMEM((QS // 2, 53 * 128), u32),
            pltpu.VMEM((4, 49, QD, 128), f32),
            pltpu.VMEM((D, S), bf16),
            pltpu.SemaphoreType.DMA((13,)),
            pltpu.SemaphoreType.DMA((NBLK,)),
            pltpu.SemaphoreType.DMA((4 * len(ECH),)),
        ],
        compiler_params=pltpu.CompilerParams(vmem_limit_bytes=110 * 1024 * 1024),
        name="adaln_blk",
    )(A_x[0].T, c, A_wqkv, A_wo, B_w1, B_w3, B_w2.T, w_mod)
    return out_t.T[None]
```

```python
import functools

import jax
import jax.numpy as jnp
import jax.experimental.pallas as pl
import jax.experimental.pallas.tpu as pltpu

S, D, F = 2048, 576, 4608
H, DH, W, DIL = 32, 18, 8, 2
EPS = 1e-5
LOG2E = 1.4426950408889634
f32, bf16, u32 = jnp.float32, jnp.bfloat16, jnp.uint32

HALO = 16
RB = 256
NBLK = S // RB
GR = 8
NQ = 1792
KM = 512
FC = 512
HD, QD, QS, QB = D // 2, D // 4, S // 4, RB // 4
MB = 23 * 128
ER = 16
ECH = (16, 32, 48, 48)
Z0, Z1 = 14, 24


def _mm(a, b):
    return jnp.dot(a, b, preferred_element_type=f32)


def _mmt(a, b):
    return jax.lax.dot_general(a, b, (((1,), (1,)), ((), ())), preferred_element_type=f32)


def _ln_t(xt):
    m = jnp.sum(xt, axis=0, keepdims=True) * (1.0 / D)
    m2 = jnp.sum(xt * xt, axis=0, keepdims=True) * (1.0 / D)
    v = jnp.maximum(m2 - m * m, 0.0)
    return (xt - m) * jax.lax.rsqrt(v + EPS)


def _swiglu(g, u):
    t = 0.5 * g
    tu = t * u
    return tu + tu * jnp.tanh(t)


def _ds(start, size):
    if isinstance(start, int):
        return pl.ds(start, size)
    return pl.ds(pl.multiple_of(start, size), size)


def _qkv_row(sec, d):
    return sec * 512 + d * 32 if d < 16 else 1536 + sec * 64 + (d - 16) * 32


def _quads(x):
    m, n = x.shape[0] // 2, x.shape[1] // 2
    return [x[:m, :n], x[:m, n:], x[m:, :n], x[m:, n:]]


def _lhs7(x):
    a, b, c, d = x
    return [a + d, c + d, a, d, a + b, c - a, b - d]


def _rhs7(x):
    a, b, c, d = x
    return [a + d, a, b - d, c - a, d, a + b, c + d]


def _rhs7n(x):
    a, b, c, d = x
    return [a + d, a, d - b, c - a, -d, a + b, c + d]


def _out4(m):
    m1, m2, m3, m4, m5, m6, m7 = m
    return [(m1 + m7) + (m4 - m5), m3 + m5, m2 + m4, (m1 + m6) + (m3 - m2)]


def _lin(terms):
    v = None
    for t, sg in terms:
        v = t if v is None else (v + t if sg > 0 else v - t)
    return v


RHS_TERMS = [[(0, 1), (3, 1)], [(0, 1)], [(1, 1), (3, -1)], [(2, 1), (0, -1)], [(3, 1)], [(0, 1), (1, 1)],
             [(2, 1), (3, 1)]]
INNER = [2, 4, 1, 3, 0, 5, 6]
OUTER = [4, 2, 1, 3, 0, 6, 5]
FIN = {2: (1, 4), 3: (2, 1), 6: (0, None), 5: (3, None)}
RIDE = {4: (1, 1), 2: (1, 3), 1: (2, 1), 3: (2, 3), 0: (0, 1), 6: (0, 3), 5: (3, 3)}
PRE = {4: [(3, 2)], 2: [(1, 0), (1, 2)], 3: [(2, 0), (2, 2)], 6: [(0, 0), (0, 2)], 5: [(3, 0), (3, 1)]}
DOWN_Q = [2, 0, 3, 1]
DOWN_IN = [4, 0, 1, 5, 2, 3, 6]
DOWN_AT = {11: [4], 19: [1, 0], 27: [2, 5, 3, 6]}


def _kernel(xt_hbm, c_hbm, wqkv_hbm, wo_hbm, w1_hbm, w3_hbm, w2t_hbm, wmod_hbm, out_hbm,
            x_v, c_v, wqkv_v, wo_v, wmod_v, w1_v, w3_v, w2t_v, tq_s, wt_s, wot_s, mod_s, gcol_s,
            part_s, q_s, kv_s, o_s, x1_s, a_s, acc_s, out_v, sems, xsems, osems):
    a_b, o_b, wt_b, wot_b = [r.bitcast(bf16) for r in (a_s, o_s, wt_s, wot_s)]

    def cp(src, dst, k):
        return pltpu.make_async_copy(src, dst, sems.at[k])

    def c_x(t):
        cols = _ds(t * RB, RB)
        return pltpu.make_async_copy(xt_hbm.at[:, cols], x_v.at[:, cols], xsems.at[t])

    c_c = cp(c_hbm, c_v, 0)
    c_ma = cp(wmod_hbm.at[:, 0:2 * D], wmod_v.at[:, 0:2 * D], 1)
    c_wq = [cp(wqkv_hbm.at[j * 128:min((j + 1) * 128, D), :], wqkv_v.at[j * 128:min((j + 1) * 128, D), :], 2 + j)
            for j in range(5)]
    c_wo = cp(wo_hbm, wo_v, 7)
    c_mb = cp(wmod_hbm.at[:, 2 * D:MB], wmod_v.at[:, 2 * D:MB], 8)
    c_mc = cp(wmod_hbm.at[:, MB:], wmod_v.at[:, MB:], 9)
    c_ffn = [cp(w1_hbm, w1_v, 10), cp(w3_hbm, w3_v, 11), cp(w2t_hbm, w2t_v, 12)]
    c_x(0).start(priority=0)
    for d in ([c_wq[0], c_c, c_ma] + c_wq[1:] + [c_wo, c_mb] + [c_x(t) for t in range(2, NBLK)]
              + [c_mc] + c_ffn):
        d.start(priority=1)

    def mod_cols(lo, hi):
        cc = c_v[...].astype(f32)
        sc = jnp.broadcast_to((cc * jax.nn.sigmoid(cc)).astype(bf16), (16, D))
        return _mm(sc, wmod_v[:, lo:hi])

    def col_bcast(row):
        return jnp.broadcast_to(row, (128, D)).T

    def modulate1(xn):
        return xn * (1.0 + mod_s[1, 0:1, :]) + mod_s[0, 0:1, :]

    def qkv_part(h1, lo, hi):
        return _mmt(h1[:, lo:hi].astype(bf16), wt_b[:, lo:hi])

    def store_qkv(qkv, par):
        rk = pl.ds(HALO, RB)
        lane = jax.lax.broadcasted_iota(jnp.int32, (RB, 128), 1)
        for j in range(4):
            q_s[par, j] = qkv[:, j * 128:(j + 1) * 128]
            kv_s[par, j, rk, :] = qkv[:, 512 + j * 128:512 + (j + 1) * 128]
            kv_s[par, 5 + j, rk, :] = qkv[:, 1024 + j * 128:1024 + (j + 1) * 128]
        t4 = qkv[:, 1536:1664]
        q_s[par, 4] = jnp.where(lane < 64, t4, 0.0)
        kv_s[par, 4, rk, :] = pltpu.roll(t4, 64, 1)
        kv_s[par, 9, rk, :] = qkv[:, 1664:1792]

    def s1(r0, par):
        kv_s[par, :, 0:HALO, :] = kv_s[1 - par, :, RB:RB + HALO, :]
        h1 = modulate1(_ln_t(x_v[:, _ds(r0, RB)].astype(f32)).T)
        tl = qkv_part(h1, KM, D)
        store_qkv(qkv_part(h1, 0, KM) + tl, par)

    def s2(par, first=False, skew=0):
        qscale = (DH ** -0.5) * LOG2E
        ngrp = RB // GR
        st = {}

        def kv(j, g, w):
            return kv_s[par, j, pl.ds(g * GR + HALO - DIL * w, GR), :]

        def scores(g):
            q = [q_s[par, j, g * GR:(g + 1) * GR, :] * qscale for j in range(5)]
            ps = []
            for w in range(W):
                p = q[0] * kv(0, g, w)
                for j in range(1, 5):
                    p = p + q[j] * kv(j, g, w)
                ps.append(p)
            p = jnp.concatenate(ps, axis=0)
            st[g] = (p, pltpu.roll(p, 64, 1))

        def fold(g):
            p, pr = st[g]
            p = p + pr
            st[g] = (p, pltpu.roll(p, 32, 1))

        def mix(g):
            p, pr = st.pop(g)
            p = p + pr
            lg = [p[w * GR:(w + 1) * GR] for w in range(W)]
            if first and g * GR < HALO:
                pos = g * GR + jax.lax.broadcasted_iota(jnp.int32, (GR, 128), 0)
                lg = [lg[0]] + [jnp.where(pos >= DIL * w, lg[w], -1e9 * LOG2E) for w in range(1, W)]
            m = jnp.maximum(jnp.maximum(jnp.maximum(lg[0], lg[1]), jnp.maximum(lg[2], lg[3])),
                            jnp.maximum(jnp.maximum(lg[4], lg[5]), jnp.maximum(lg[6], lg[7])))
            e = [jnp.exp2(l - m) for l in lg]
            den = ((e[0] + e[1]) + (e[2] + e[3])) + ((e[4] + e[5]) + (e[6] + e[7]))
            inv = pl.reciprocal(den, approx=True)
            inv = inv * (2.0 - den * inv)
            for j in range(5):
                a = e[0] * kv(5 + j, g, 0)
                for w in range(1, W):
                    a = a + e[w] * kv(5 + j, g, w)
                if g % 2 == 0:
                    st[('o', j)] = a * inv
                else:
                    both = jnp.concatenate([st.pop(('o', j)), a * inv], axis=0)
                    o_b[(g - 1) * GR:(g + 1) * GR, (par * 5 + j) * 128:(par * 5 + j + 1) * 128] = both.astype(bf16)

        for i in range(ngrp + 2 * skew):
            if i < ngrp:
                scores(i)
            if 0 <= i - skew < ngrp:
                fold(i - skew)
            if 0 <= i - 2 * skew < ngrp:
                mix(i - 2 * skew)

    def s3(r0, par):
        r = _ds(r0, RB)
        att = _mmt(wot_b[...], o_b[:, par * 640:(par + 1) * 640])
        ga = jnp.concatenate([gcol_s[0]] * (RB // 128), axis=1)
        x1 = x_v[:, r].astype(f32) + ga * att
        x1_s[:, r] = x1
        h = _ln_t(x1).T * (1.0 + mod_s[3, 0:1, :]) + mod_s[2, 0:1, :]
        rr = _ds(r0 // 4, QB)
        for ka, y in enumerate(_lhs7(_quads(h[:, 0:KM]))):
            for kb, z in enumerate(_lhs7(_quads(y))):
                a_b[rr, (ka * 7 + kb) * 128:(ka * 7 + kb + 1) * 128] = z.astype(bf16)
        for i in range(4):
            a_b[rr, (49 + i) * 128:(49 + i) * 128 + 64] = h[i * QB:(i + 1) * QB, KM:D].astype(bf16)

    def prep_wq(j):
        w = 128 if j < 4 else 64
        tq_s[j, :, 0:w] = wqkv_v[j * 128:j * 128 + w, :].astype(f32).T
        for sec in range(3):
            for d in range(DH):
                g = tq_s[j, pl.ds(sec * D + d, H, stride=DH), :]
                dst = _qkv_row(sec, d)
                wt_b[dst:dst + 32, j * 128:j * 128 + w] = g[:, 0:w].astype(bf16)

    def prep_wo():
        for j in range(5):
            w = 128 if j < 4 else 64
            tq_s[j, 0:D, 0:w] = wo_v[:, j * 128:j * 128 + w].astype(f32)
        for j in range(5):
            w = 128 if j < 4 else 64
            parts = [tq_s[j, pl.ds(d, H, stride=DH), :] for d in range(DH)] + [jnp.zeros((64, 128), f32)]
            wot_b[j * 128:j * 128 + w, :] = jnp.concatenate(parts, axis=0).T[0:w, :].astype(bf16)

    def clear(k, carry):
        acc_s[k // 7, pl.ds((k % 7) * 7, 7)] = jnp.zeros((7, QD, 128), f32)
        return carry

    kv_s[0, :, 0:HALO, :] = jnp.zeros((10, HALO, 128), f32)
    wt_b[3 * D:NQ, :] = jnp.zeros((NQ - 3 * D, 640), bf16)
    tq_s[4] = jnp.zeros((3 * D, 128), f32)
    jax.lax.fori_loop(0, Z0, clear, 0)
    c_x(0).wait()
    c_wq[0].wait()
    xn = _ln_t(x_v[:, 0:RB].astype(f32)).T
    prep_wq(0)
    jax.lax.fori_loop(Z0, Z1, clear, 0)
    c_c.wait()
    c_ma.wait()
    mod = mod_cols(0, 2 * D)
    mod_s[0] = mod[0:8, 0:D]
    mod_s[1] = mod[0:8, D:2 * D]
    h1 = modulate1(xn)
    c_wq[1].wait()
    c_x(1).start(priority=0)
    part_s[...] = qkv_part(h1, 0, 128)
    prep_wq(1)
    c_wq[2].wait()
    part_s[...] += qkv_part(h1, 128, 256)
    prep_wq(2)
    c_wq[3].wait()
    c_wq[4].wait()
    c_x(1).wait()
    part = part_s[...] + qkv_part(h1, 256, 384)
    prep_wq(3)
    prep_wq(4)
    store_qkv(part + qkv_part(h1, 384, D), 0)
    o_b[:, 640:640 + D] = modulate1(_ln_t(x_v[:, RB:2 * RB].astype(f32)).T).astype(bf16)

    c_wo.wait()
    prep_wo()
    kv_s[1, :, 0:HALO, :] = kv_s[0, :, RB:RB + HALO, :]
    tl = _mmt(o_b[:, 640 + KM:640 + D], wt_b[:, KM:D])
    store_qkv(_mmt(o_b[:, 640:640 + KM], wt_b[:, 0:KM]) + tl, 1)
    s2(0, first=True, skew=1)
    c_mb.wait()
    mod = mod_cols(2 * D, MB)
    gcol_s[0] = col_bcast(mod[0:1, 0:D])
    mod_s[2] = mod[0:8, D:2 * D]
    mod_s[3] = mod[0:8, 2 * D:3 * D]
    acc_s[3, (Z1 - 21) * 7:49] = jnp.zeros(((28 - Z1) * 7, QD, 128), f32)

    def a_step(t, par):
        s3((t - 2) * RB, par)
        s1(t * RB, par)
        s2(1 - par)

    def a_body(t, carry):
        c_x(t).wait()
        for par in range(2):
            pl.when(t % 2 == par)(functools.partial(a_step, t, par))
        return carry

    jax.lax.fori_loop(2, NBLK, a_body, 0)

    c_mc.wait()
    gcol_s[1] = col_bcast(mod_cols(MB - 128, 6 * D)[0:1, 64:64 + D])
    s3(S - 2 * RB, 0)
    s2(1)
    s3(S - RB, 1)
    for d in c_ffn:
        d.wait()

    def b_body(ci, carry):
        n = _ds(ci * FC, FC)
        w_out = [_rhs7(_quads(w[0:KM, n].astype(f32))) for w in (w1_v, w3_v)]
        w_tail = [w[KM:D, n] for w in (w1_v, w3_v)]
        w2_out = _lhs7(_quads(w2t_v[:, n].astype(f32)))
        tails, mo, gate, psum = [{}, {}], [[None] * 7, [None] * 7], {}, [{}, {}]
        hid, hblk = {}, {}

        def tail(x, oq, iq):
            i, j = (oq // 2) * 2 + iq // 2, (oq % 2) * 2 + iq % 2
            return _mm(a_b[:, (49 + i) * 128:(49 + i) * 128 + 64], w_tail[x][:, j * 128:(j + 1) * 128])

        def chain(x, v, terms, iq):
            for k, sg in terms:
                v = v + mo[x][k][iq] if (sg > 0) != (iq == 1) else v - mo[x][k][iq]
            return v

        def final(x, a, iq):
            if a == 0:
                m1 = mo[x][0][iq] if iq != 1 else -mo[x][0][iq]
                psum[x][(0, iq)] = chain(x, m1, [(3, 1), (4, -1)], iq)
                psum[x][(3, iq)] = chain(x, m1, [(2, 1), (1, -1)], iq)
            if a not in FIN:
                return
            oq, partner = FIN[a]
            if partner is None:
                v = chain(x, tails[x][(oq, iq)], [(a, 1)], iq) + psum[x][(oq, iq)]
            else:
                v = chain(x, tails[x][(oq, iq)], [(a, 1), (partner, 1)], iq)
            if x == 0:
                gate[(oq, iq)] = v
            else:
                hid[(oq, iq)] = _swiglu(gate[(oq, iq)], v)

        def hidden(oq, j):
            if (oq, j) not in hblk:
                kk, nn = divmod(j, 2)
                parts = []
                for t in range(4):
                    rs = slice((2 * t + nn) * QB, (2 * t + nn + 1) * QB)
                    parts += [hid[(oq, kk)][rs], hid[(oq, 2 + kk)][rs]]
                hblk[(oq, j)] = jnp.concatenate(parts, axis=0)
            return hblk[(oq, j)]

        def down(wave):
            for a in DOWN_AT.get(wave, []):
                lhs = [z.astype(bf16) for z in _lhs7(_quads(w2_out[a]))]
                for b in DOWN_IN:
                    terms = [(hidden(DOWN_Q[i], j), si * sj) for i, si in RHS_TERMS[a] for j, sj in RHS_TERMS[b]]
                    if len(terms) == 4:
                        terms = [terms[0], terms[3], terms[1], terms[2]]
                    r = _mmt(lhs[b], _lin(terms).astype(bf16))
                    for t in range(4):
                        acc_s[t, a * 7 + b] += r[:, t * 128:(t + 1) * 128]

        wave = 0
        for a in OUTER:
            for x in range(2):
                for key in PRE.get(a, []):
                    tails[x][key] = tail(x, *key)
            for x in range(2):
                rhs = [z.astype(bf16) for z in _rhs7n(_quads(w_out[x][a]))]
                m = [None] * 7
                for b in INNER[:4]:
                    m[b] = _mm(a_b[:, (a * 7 + b) * 128:(a * 7 + b + 1) * 128], rhs[b])
                sa = [m[3] + m[4], m[2] + m[4], m[1] + m[3], m[2] + m[1]]
                mo[x][a] = [None, sa[1], sa[2], None]
                final(x, a, 1)
                final(x, a, 2)
                down(wave)
                for b in INNER[4:]:
                    m[b] = _mm(a_b[:, (a * 7 + b) * 128:(a * 7 + b + 1) * 128], rhs[b])
                tails[x][RIDE[a]] = tail(x, *RIDE[a])
                mo[x][a] = [(m[0] + m[6]) + sa[0], sa[1], sa[2], (m[0] + m[5]) - sa[3]]
                final(x, a, 0)
                final(x, a, 3)
                down(wave + 1)
                wave += 2
        return carry

    jax.lax.fori_loop(0, F // FC, b_body, 0)

    copies = []
    r0 = 0
    for ck, rows in enumerate(ECH):
        for r in range(r0, r0 + rows, ER):
            for t in range(4):
                cs = slice(t * QS, (t + 1) * QS)
                mo = [_out4([acc_s[t, a * 7 + b, r:r + ER, :] for b in range(7)]) for a in range(7)]
                cq = [_out4([mo[a][i] for a in range(7)]) for i in range(4)]
                for mq in range(4):
                    rs = slice(mq * QD + r, mq * QD + r + ER)
                    row = jnp.concatenate([cq[(mq % 2) * 2 + nn][(mq // 2) * 2 + 1 - hh]
                                           for nn in range(2) for hh in range(2)], axis=1)
                    gb = jnp.concatenate([gcol_s[1, rs, :]] * 4, axis=1)
                    out_v[rs, cs] = (x1_s[rs, cs] + gb * row).astype(bf16)
        for mq in range(4):
            rs = slice(mq * QD + r0, mq * QD + r0 + rows)
            d = pltpu.make_async_copy(out_v.at[rs, :], out_hbm.at[rs, :], osems.at[ck * 4 + mq])
            d.start()
            copies.append(d)
        r0 += rows
    for d in copies:
        d.wait()


@jax.jit
def pallas_adaLN_cond__sliding_local_dilated__glu_gated_swiglu__prompt_kernel(
    A_x: jax.Array,
    A_wqkv: jax.Array,
    A_wo: jax.Array,
    B_x: jax.Array,
    B_w1: jax.Array,
    B_w3: jax.Array,
    B_w2: jax.Array,
    c: jax.Array,
    w_mod: jax.Array,
):
    del B_x
    hbm = pl.BlockSpec(memory_space=pl.ANY)
    out_t = pl.pallas_call(
        _kernel,
        in_specs=[hbm] * 8,
        out_specs=hbm,
        out_shape=jax.ShapeDtypeStruct((D, S), bf16),
        scratch_shapes=[
            pltpu.VMEM((D, S), bf16),
            pltpu.VMEM((1, D), bf16),
            pltpu.VMEM((D, 3 * D), bf16),
            pltpu.VMEM((D, D), bf16),
            pltpu.VMEM((D, 6 * D), bf16),
            pltpu.VMEM((D, F), bf16),
            pltpu.VMEM((D, F), bf16),
            pltpu.VMEM((D, F), bf16),
            pltpu.VMEM((5, 3 * D, 128), f32),
            pltpu.VMEM((NQ // 2, 640), u32),
            pltpu.VMEM((D // 2, 640), u32),
            pltpu.VMEM((4, 8, D), f32),
            pltpu.VMEM((2, D, 128), f32),
            pltpu.VMEM((RB, NQ), f32),
            pltpu.VMEM((2, 5, RB, 128), f32),
            pltpu.VMEM((2, 10, RB + HALO, 128), f32),
            pltpu.VMEM((RB // 2, 2 * 640), u32),
            pltpu.VMEM((D, S), f32),
            pltpu.VMEM((QS // 2, 53 * 128), u32),
            pltpu.VMEM((4, 49, QD, 128), f32),
            pltpu.VMEM((D, S), bf16),
            pltpu.SemaphoreType.DMA((13,)),
            pltpu.SemaphoreType.DMA((NBLK,)),
            pltpu.SemaphoreType.DMA((4 * len(ECH),)),
        ],
        compiler_params=pltpu.CompilerParams(vmem_limit_bytes=110 * 1024 * 1024),
        name="adaln_blk",
    )(A_x[0].T, c, A_wqkv, A_wo, B_w1, B_w3, B_w2.T, w_mod)
    return out_t.T[None]
```

```python
import functools

import jax
import jax.numpy as jnp
import jax.experimental.pallas as pl
import jax.experimental.pallas.tpu as pltpu

S, D, F = 2048, 576, 4608
H, DH, W, DIL = 32, 18, 8, 2
EPS = 1e-5
LOG2E = 1.4426950408889634
f32, bf16, u32 = jnp.float32, jnp.bfloat16, jnp.uint32

HALO = 16
RB = 256
NBLK = S // RB
GR = 8
NQ = 1792
KM = 512
FC = 512
HD, QD, QS, QB = D // 2, D // 4, S // 4, RB // 4
MB = 23 * 128
ER = 16
ECH = (16, 32, 48, 48)
Z0, Z1 = 14, 24


def _mm(a, b):
    return jnp.dot(a, b, preferred_element_type=f32)


def _mmt(a, b):
    return jax.lax.dot_general(a, b, (((1,), (1,)), ((), ())), preferred_element_type=f32)


def _ln_t(xt):
    m = jnp.sum(xt, axis=0, keepdims=True) * (1.0 / D)
    m2 = jnp.sum(xt * xt, axis=0, keepdims=True) * (1.0 / D)
    v = jnp.maximum(m2 - m * m, 0.0)
    return (xt - m) * jax.lax.rsqrt(v + EPS)


def _swiglu(g, u):
    t = 0.5 * g
    tu = t * u
    return tu + tu * jnp.tanh(t)


def _ds(start, size):
    if isinstance(start, int):
        return pl.ds(start, size)
    return pl.ds(pl.multiple_of(start, size), size)


def _qkv_row(sec, d):
    return sec * 512 + d * 32 if d < 16 else 1536 + sec * 64 + (d - 16) * 32


def _quads(x):
    m, n = x.shape[0] // 2, x.shape[1] // 2
    return [x[:m, :n], x[:m, n:], x[m:, :n], x[m:, n:]]


def _lhs7(x):
    a, b, c, d = x
    return [a + d, c + d, a, d, a + b, c - a, b - d]


def _rhs7(x):
    a, b, c, d = x
    return [a + d, a, b - d, c - a, d, a + b, c + d]


def _rhs7n(x):
    a, b, c, d = x
    return [a + d, a, d - b, c - a, -d, a + b, c + d]


def _out4(m):
    m1, m2, m3, m4, m5, m6, m7 = m
    return [(m1 + m7) + (m4 - m5), m3 + m5, m2 + m4, (m1 + m6) + (m3 - m2)]


def _lin(terms):
    v = None
    for t, sg in terms:
        v = t if v is None else (v + t if sg > 0 else v - t)
    return v


RHS_TERMS = [[(0, 1), (3, 1)], [(0, 1)], [(1, 1), (3, -1)], [(2, 1), (0, -1)], [(3, 1)], [(0, 1), (1, 1)],
             [(2, 1), (3, 1)]]
INNER = [2, 4, 1, 3, 0, 5, 6]
OUTER = [4, 2, 1, 3, 0, 6, 5]
FIN = {2: (1, 4), 3: (2, 1), 6: (0, None), 5: (3, None)}
RIDE = {4: (1, 1), 2: (1, 3), 1: (2, 1), 3: (2, 3), 0: (0, 1), 6: (0, 3), 5: (3, 3)}
PRE = {4: [(3, 2)], 2: [(1, 0), (1, 2)], 3: [(2, 0), (2, 2)], 6: [(0, 0), (0, 2)], 5: [(3, 0), (3, 1)]}
DOWN_Q = [2, 0, 3, 1]
DOWN_IN = [4, 0, 1, 5, 2, 3, 6]
DOWN_AT = {11: [4], 19: [1, 0], 27: [2, 5, 3, 6]}


def _kernel(xt_hbm, c_hbm, wqkv_hbm, wo_hbm, w1_hbm, w3_hbm, w2t_hbm, wmod_hbm, out_hbm,
            x_v, c_v, wqkv_v, wo_v, wmod_v, w1_v, w3_v, w2t_v, tq_s, wt_s, wot_s, mod_s, gcol_s,
            part_s, q_s, kv_s, o_s, x1_s, a_s, acc_s, out_v, sems, xsems, osems):
    a_b, o_b, wt_b, wot_b = [r.bitcast(bf16) for r in (a_s, o_s, wt_s, wot_s)]

    def cp(src, dst, k):
        return pltpu.make_async_copy(src, dst, sems.at[k])

    def c_x(t):
        return pltpu.make_async_copy(xt_hbm.at[:, _ds(t * RB, RB)], x_v.at[t], xsems.at[t])

    c_c = cp(c_hbm, c_v, 0)
    c_ma = cp(wmod_hbm.at[:, 0:2 * D], wmod_v.at[:, 0:2 * D], 1)
    c_wq = [cp(wqkv_hbm.at[j * 128:min((j + 1) * 128, D), :], wqkv_v.at[j * 128:min((j + 1) * 128, D), :], 2 + j)
            for j in range(5)]
    c_wo = cp(wo_hbm, wo_v, 7)
    c_mb = cp(wmod_hbm.at[:, 2 * D:MB], wmod_v.at[:, 2 * D:MB], 8)
    c_mc = cp(wmod_hbm.at[:, MB:], wmod_v.at[:, MB:], 9)
    c_ffn = [cp(w1_hbm, w1_v, 10), cp(w3_hbm, w3_v, 11), cp(w2t_hbm, w2t_v, 12)]
    c_x(0).start(priority=0)
    for d in ([c_wq[0], c_c, c_ma] + c_wq[1:] + [c_wo, c_mb] + [c_x(t) for t in range(2, NBLK)]
              + [c_mc] + c_ffn):
        d.start(priority=1)

    def mod_cols(lo, hi):
        cc = c_v[...].astype(f32)
        sc = jnp.broadcast_to((cc * jax.nn.sigmoid(cc)).astype(bf16), (16, D))
        return _mm(sc, wmod_v[:, lo:hi])

    def col_bcast(row):
        return jnp.broadcast_to(row, (128, D)).T

    def modulate1(xn):
        return xn * (1.0 + mod_s[1, 0:1, :]) + mod_s[0, 0:1, :]

    def qkv_part(h1, lo, hi):
        return _mmt(h1[:, lo:hi].astype(bf16), wt_b[:, lo:hi])

    def store_qkv(qkv, par):
        rk = pl.ds(HALO, RB)
        lane = jax.lax.broadcasted_iota(jnp.int32, (RB, 128), 1)
        for j in range(4):
            q_s[par, j] = qkv[:, j * 128:(j + 1) * 128]
            kv_s[par, j, rk, :] = qkv[:, 512 + j * 128:512 + (j + 1) * 128]
            kv_s[par, 5 + j, rk, :] = qkv[:, 1024 + j * 128:1024 + (j + 1) * 128]
        t4 = qkv[:, 1536:1664]
        q_s[par, 4] = jnp.where(lane < 64, t4, 0.0)
        kv_s[par, 4, rk, :] = pltpu.roll(t4, 64, 1)
        kv_s[par, 9, rk, :] = qkv[:, 1664:1792]

    def s1(t, par):
        kv_s[par, :, 0:HALO, :] = kv_s[1 - par, :, RB:RB + HALO, :]
        h1 = modulate1(_ln_t(x_v[t].astype(f32)).T)
        tl = qkv_part(h1, KM, D)
        store_qkv(qkv_part(h1, 0, KM) + tl, par)

    def s2(par, first=False, skew=0):
        qscale = (DH ** -0.5) * LOG2E
        ngrp = RB // GR
        st = {}

        def kv(j, g, w):
            return kv_s[par, j, pl.ds(g * GR + HALO - DIL * w, GR), :]

        def scores(g):
            q = [q_s[par, j, g * GR:(g + 1) * GR, :] * qscale for j in range(5)]
            ps = []
            for w in range(W):
                p = q[0] * kv(0, g, w)
                for j in range(1, 5):
                    p = p + q[j] * kv(j, g, w)
                ps.append(p)
            p = jnp.concatenate(ps, axis=0)
            st[g] = (p, pltpu.roll(p, 64, 1))

        def fold(g):
            p, pr = st[g]
            p = p + pr
            st[g] = (p, pltpu.roll(p, 32, 1))

        def mix(g):
            p, pr = st.pop(g)
            p = p + pr
            lg = [p[w * GR:(w + 1) * GR] for w in range(W)]
            if first and g * GR < HALO:
                pos = g * GR + jax.lax.broadcasted_iota(jnp.int32, (GR, 128), 0)
                lg = [lg[0]] + [jnp.where(pos >= DIL * w, lg[w], -1e9 * LOG2E) for w in range(1, W)]
            m = jnp.maximum(jnp.maximum(jnp.maximum(lg[0], lg[1]), jnp.maximum(lg[2], lg[3])),
                            jnp.maximum(jnp.maximum(lg[4], lg[5]), jnp.maximum(lg[6], lg[7])))
            e = [jnp.exp2(l - m) for l in lg]
            den = ((e[0] + e[1]) + (e[2] + e[3])) + ((e[4] + e[5]) + (e[6] + e[7]))
            inv = pl.reciprocal(den, approx=True)
            inv = inv * (2.0 - den * inv)
            for j in range(5):
                a = e[0] * kv(5 + j, g, 0)
                for w in range(1, W):
                    a = a + e[w] * kv(5 + j, g, w)
                if g % 2 == 0:
                    st[('o', j)] = a * inv
                else:
                    both = jnp.concatenate([st.pop(('o', j)), a * inv], axis=0)
                    o_b[(g - 1) * GR:(g + 1) * GR, (par * 5 + j) * 128:(par * 5 + j + 1) * 128] = both.astype(bf16)

        for i in range(ngrp + 2 * skew):
            if i < ngrp:
                scores(i)
            if 0 <= i - skew < ngrp:
                fold(i - skew)
            if 0 <= i - 2 * skew < ngrp:
                mix(i - 2 * skew)

    def s3(t, par):
        att = _mmt(wot_b[...], o_b[:, par * 640:(par + 1) * 640])
        ga = jnp.concatenate([gcol_s[0]] * (RB // 128), axis=1)
        x1 = x_v[t].astype(f32) + ga * att
        x1_s[:, _ds(t * RB, RB)] = x1
        h = _ln_t(x1).T * (1.0 + mod_s[3, 0:1, :]) + mod_s[2, 0:1, :]
        rr = _ds(t * QB, QB)
        for ka, y in enumerate(_lhs7(_quads(h[:, 0:KM]))):
            for kb, z in enumerate(_lhs7(_quads(y))):
                a_b[rr, (ka * 7 + kb) * 128:(ka * 7 + kb + 1) * 128] = z.astype(bf16)
        for i in range(4):
            a_b[rr, (49 + i) * 128:(49 + i) * 128 + 64] = h[i * QB:(i + 1) * QB, KM:D].astype(bf16)

    def prep_wq(j):
        w = 128 if j < 4 else 64
        tq_s[j, 0:3 * D, 0:w] = wqkv_v[j * 128:j * 128 + w, :].astype(f32).T
        for sec in range(3):
            for d in range(DH):
                g = tq_s[j, pl.ds(sec * D + d, H, stride=DH), :]
                dst = _qkv_row(sec, d)
                wt_b[dst:dst + 32, j * 128:j * 128 + w] = g[:, 0:w].astype(bf16)

    def prep_wo():
        for j in range(5):
            w = 128 if j < 4 else 64
            tq_s[j, 0:D, 0:w] = wo_v[:, j * 128:j * 128 + w].astype(f32)
        for j in range(5):
            w = 128 if j < 4 else 64
            parts = [tq_s[j, pl.ds(d, H, stride=DH), :] for d in range(DH)] + [jnp.zeros((64, 128), f32)]
            wot_b[j * 128:j * 128 + w, :] = jnp.concatenate(parts, axis=0).T[0:w, :].astype(bf16)

    def clear(k, carry):
        acc_s[k // 7, pl.ds((k % 7) * 7, 7)] = jnp.zeros((7, QD, 128), f32)
        return carry

    kv_s[0, :, 0:HALO, :] = jnp.zeros((10, HALO, 128), f32)
    wt_b[3 * D:NQ, :] = jnp.zeros((NQ - 3 * D, 640), bf16)
    tq_s[0:4, 3 * D:, :] = jnp.zeros((4, 24, 128), f32)
    tq_s[4] = jnp.zeros((3 * D + 24, 128), f32)
    jax.lax.fori_loop(0, Z0, clear, 0)
    c_x(0).wait()
    c_wq[0].wait()
    xn = _ln_t(x_v[0].astype(f32)).T
    prep_wq(0)
    jax.lax.fori_loop(Z0, Z1, clear, 0)
    c_c.wait()
    c_ma.wait()
    mod = mod_cols(0, 2 * D)
    mod_s[0] = mod[0:8, 0:D]
    mod_s[1] = mod[0:8, D:2 * D]
    h1 = modulate1(xn)
    c_wq[1].wait()
    c_x(1).start(priority=0)
    part_s[...] = qkv_part(h1, 0, 128)
    prep_wq(1)
    c_wq[2].wait()
    part_s[...] += qkv_part(h1, 128, 256)
    prep_wq(2)
    c_wq[3].wait()
    c_wq[4].wait()
    c_x(1).wait()
    part = part_s[...] + qkv_part(h1, 256, 384)
    prep_wq(3)
    prep_wq(4)
    store_qkv(part + qkv_part(h1, 384, D), 0)
    o_b[:, 640:640 + D] = modulate1(_ln_t(x_v[1].astype(f32)).T).astype(bf16)

    c_wo.wait()
    prep_wo()
    kv_s[1, :, 0:HALO, :] = kv_s[0, :, RB:RB + HALO, :]
    tl = _mmt(o_b[:, 640 + KM:640 + D], wt_b[:, KM:D])
    store_qkv(_mmt(o_b[:, 640:640 + KM], wt_b[:, 0:KM]) + tl, 1)
    s2(0, first=True, skew=1)
    c_mb.wait()
    mod = mod_cols(2 * D, MB)
    gcol_s[0] = col_bcast(mod[0:1, 0:D])
    mod_s[2] = mod[0:8, D:2 * D]
    mod_s[3] = mod[0:8, 2 * D:3 * D]
    acc_s[3, (Z1 - 21) * 7:49] = jnp.zeros(((28 - Z1) * 7, QD, 128), f32)

    def a_step(t, par):
        s3(t - 2, par)
        s1(t, par)
        s2(1 - par)

    def a_body(t, carry):
        c_x(t).wait()
        for par in range(2):
            pl.when(t % 2 == par)(functools.partial(a_step, t, par))
        return carry

    jax.lax.fori_loop(2, NBLK, a_body, 0)

    c_mc.wait()
    gcol_s[1] = col_bcast(mod_cols(MB - 128, 6 * D)[0:1, 64:64 + D])
    s3(NBLK - 2, 0)
    s2(1)
    s3(NBLK - 1, 1)
    for d in c_ffn:
        d.wait()

    def b_body(ci, carry):
        n = _ds(ci * FC, FC)
        w_out = [_rhs7(_quads(w[0:KM, n].astype(f32))) for w in (w1_v, w3_v)]
        w_tail = [w[KM:D, n] for w in (w1_v, w3_v)]
        w2_out = _lhs7(_quads(w2t_v[:, n].astype(f32)))
        tails, mo, gate, psum = [{}, {}], [[None] * 7, [None] * 7], {}, [{}, {}]
        hid, hblk = {}, {}

        def tail(x, oq, iq):
            i, j = (oq // 2) * 2 + iq // 2, (oq % 2) * 2 + iq % 2
            return _mm(a_b[:, (49 + i) * 128:(49 + i) * 128 + 64], w_tail[x][:, j * 128:(j + 1) * 128])

        def chain(x, v, terms, iq):
            for k, sg in terms:
                v = v + mo[x][k][iq] if (sg > 0) != (iq == 1) else v - mo[x][k][iq]
            return v

        def final(x, a, iq):
            if a == 0:
                m1 = mo[x][0][iq] if iq != 1 else -mo[x][0][iq]
                psum[x][(0, iq)] = chain(x, m1, [(3, 1), (4, -1)], iq)
                psum[x][(3, iq)] = chain(x, m1, [(2, 1), (1, -1)], iq)
            if a not in FIN:
                return
            oq, partner = FIN[a]
            if partner is None:
                v = chain(x, tails[x][(oq, iq)], [(a, 1)], iq) + psum[x][(oq, iq)]
            else:
                v = chain(x, tails[x][(oq, iq)], [(a, 1), (partner, 1)], iq)
            if x == 0:
                gate[(oq, iq)] = v
            else:
                hid[(oq, iq)] = _swiglu(gate[(oq, iq)], v)

        def hidden(oq, j):
            if (oq, j) not in hblk:
                kk, nn = divmod(j, 2)
                parts = []
                for t in range(4):
                    rs = slice((2 * t + nn) * QB, (2 * t + nn + 1) * QB)
                    parts += [hid[(oq, kk)][rs], hid[(oq, 2 + kk)][rs]]
                hblk[(oq, j)] = jnp.concatenate(parts, axis=0)
            return hblk[(oq, j)]

        def down(wave):
            for a in DOWN_AT.get(wave, []):
                lhs = [z.astype(bf16) for z in _lhs7(_quads(w2_out[a]))]
                for b in DOWN_IN:
                    terms = [(hidden(DOWN_Q[i], j), si * sj) for i, si in RHS_TERMS[a] for j, sj in RHS_TERMS[b]]
                    if len(terms) == 4:
                        terms = [terms[0], terms[3], terms[1], terms[2]]
                    r = _mmt(lhs[b], _lin(terms).astype(bf16))
                    for t in range(4):
                        acc_s[t, a * 7 + b] += r[:, t * 128:(t + 1) * 128]

        wave = 0
        for a in OUTER:
            for x in range(2):
                for key in PRE.get(a, []):
                    tails[x][key] = tail(x, *key)
            for x in range(2):
                rhs = [z.astype(bf16) for z in _rhs7n(_quads(w_out[x][a]))]
                m = [None] * 7
                for b in INNER[:4]:
                    m[b] = _mm(a_b[:, (a * 7 + b) * 128:(a * 7 + b + 1) * 128], rhs[b])
                sa = [m[3] + m[4], m[2] + m[4], m[1] + m[3], m[2] + m[1]]
                mo[x][a] = [None, sa[1], sa[2], None]
                final(x, a, 1)
                final(x, a, 2)
                down(wave)
                for b in INNER[4:]:
                    m[b] = _mm(a_b[:, (a * 7 + b) * 128:(a * 7 + b + 1) * 128], rhs[b])
                tails[x][RIDE[a]] = tail(x, *RIDE[a])
                mo[x][a] = [(m[0] + m[6]) + sa[0], sa[1], sa[2], (m[0] + m[5]) - sa[3]]
                final(x, a, 0)
                final(x, a, 3)
                down(wave + 1)
                wave += 2
        return carry

    jax.lax.fori_loop(0, F // FC, b_body, 0)

    copies = []
    r0 = 0
    for ck, rows in enumerate(ECH):
        for r in range(r0, r0 + rows, ER):
            for t in range(4):
                cs = slice(t * QS, (t + 1) * QS)
                mo = [_out4([acc_s[t, a * 7 + b, r:r + ER, :] for b in range(7)]) for a in range(7)]
                cq = [_out4([mo[a][i] for a in range(7)]) for i in range(4)]
                for mq in range(4):
                    rs = slice(mq * QD + r, mq * QD + r + ER)
                    row = jnp.concatenate([cq[(mq % 2) * 2 + nn][(mq // 2) * 2 + 1 - hh]
                                           for nn in range(2) for hh in range(2)], axis=1)
                    gb = jnp.concatenate([gcol_s[1, rs, :]] * 4, axis=1)
                    out_v[rs, cs] = (x1_s[rs, cs] + gb * row).astype(bf16)
        for mq in range(4):
            rs = slice(mq * QD + r0, mq * QD + r0 + rows)
            d = pltpu.make_async_copy(out_v.at[rs, :], out_hbm.at[rs, :], osems.at[ck * 4 + mq])
            d.start()
            copies.append(d)
        r0 += rows
    for d in copies:
        d.wait()


@jax.jit
def pallas_adaLN_cond__sliding_local_dilated__glu_gated_swiglu__prompt_kernel(
    A_x: jax.Array,
    A_wqkv: jax.Array,
    A_wo: jax.Array,
    B_x: jax.Array,
    B_w1: jax.Array,
    B_w3: jax.Array,
    B_w2: jax.Array,
    c: jax.Array,
    w_mod: jax.Array,
):
    del B_x
    hbm = pl.BlockSpec(memory_space=pl.ANY)
    out_t = pl.pallas_call(
        _kernel,
        in_specs=[hbm] * 8,
        out_specs=hbm,
        out_shape=jax.ShapeDtypeStruct((D, S), bf16),
        scratch_shapes=[
            pltpu.VMEM((NBLK, D, RB), bf16),
            pltpu.VMEM((1, D), bf16),
            pltpu.VMEM((D, 3 * D), bf16),
            pltpu.VMEM((D, D), bf16),
            pltpu.VMEM((D, 6 * D), bf16),
            pltpu.VMEM((D, F), bf16),
            pltpu.VMEM((D, F), bf16),
            pltpu.VMEM((D, F), bf16),
            pltpu.VMEM((5, 3 * D + 24, 128), f32),
            pltpu.VMEM((NQ // 2, 640), u32),
            pltpu.VMEM((D // 2, 640), u32),
            pltpu.VMEM((4, 8, D), f32),
            pltpu.VMEM((2, D, 128), f32),
            pltpu.VMEM((RB, NQ), f32),
            pltpu.VMEM((2, 5, RB, 128), f32),
            pltpu.VMEM((2, 10, RB + HALO, 128), f32),
            pltpu.VMEM((RB // 2, 2 * 640), u32),
            pltpu.VMEM((D, S), f32),
            pltpu.VMEM((QS // 2, 53 * 128), u32),
            pltpu.VMEM((4, 49, QD, 128), f32),
            pltpu.VMEM((D, S), bf16),
            pltpu.SemaphoreType.DMA((13,)),
            pltpu.SemaphoreType.DMA((NBLK,)),
            pltpu.SemaphoreType.DMA((4 * len(ECH),)),
        ],
        compiler_params=pltpu.CompilerParams(vmem_limit_bytes=110 * 1024 * 1024),
        name="adaln_blk",
    )(A_x[0].T, c, A_wqkv, A_wo, B_w1, B_w3, B_w2.T, w_mod)
    return out_t.T[None]
```

```python
import functools

import jax
import jax.numpy as jnp
import jax.experimental.pallas as pl
import jax.experimental.pallas.tpu as pltpu

S, D, F = 2048, 576, 4608
H, DH, W, DIL = 32, 18, 8, 2
EPS = 1e-5
LOG2E = 1.4426950408889634
f32, bf16, u32 = jnp.float32, jnp.bfloat16, jnp.uint32

HALO = 16
RB = 256
NBLK = S // RB
GR = 8
NQ = 1792
KM = 512
FC = 512
QD, QS, QB = D // 4, S // 4, RB // 4
MB = 23 * 128
ER = 16
ECH = (16, 32, 48, 48)
Z0, Z1 = 13, 23


def _mm(a, b):
    return jnp.dot(a, b, preferred_element_type=f32)


def _mmt(a, b):
    return jax.lax.dot_general(a, b, (((1,), (1,)), ((), ())), preferred_element_type=f32)


def _ln_t(xt):
    m = jnp.sum(xt, axis=0, keepdims=True) * (1.0 / D)
    m2 = jnp.sum(xt * xt, axis=0, keepdims=True) * (1.0 / D)
    v = jnp.maximum(m2 - m * m, 0.0)
    return (xt - m) * jax.lax.rsqrt(v + EPS)


def _swiglu(g, u):
    t = 0.5 * g
    tu = t * u
    return tu + tu * jnp.tanh(t)


def _ds(start, size):
    if isinstance(start, int):
        return pl.ds(start, size)
    return pl.ds(pl.multiple_of(start, size), size)


def _qkv_row(sec, d):
    return sec * 512 + d * 32 if d < 16 else 1536 + sec * 64 + (d - 16) * 32


def _quads(x):
    m, n = x.shape[0] // 2, x.shape[1] // 2
    return [x[:m, :n], x[:m, n:], x[m:, :n], x[m:, n:]]


def _lhs7(x):
    a, b, c, d = x
    return [a + d, c + d, a, d, a + b, c - a, b - d]


def _rhs7(x):
    a, b, c, d = x
    return [a + d, a, b - d, c - a, d, a + b, c + d]


def _rhs7n(x):
    a, b, c, d = x
    return [a + d, a, d - b, c - a, -d, a + b, c + d]


def _out4(m):
    m1, m2, m3, m4, m5, m6, m7 = m
    return [(m1 + m7) + (m4 - m5), m3 + m5, m2 + m4, (m1 + m6) + (m3 - m2)]


def _lin(terms):
    v = None
    for t, sg in terms:
        v = t if v is None else (v + t if sg > 0 else v - t)
    return v


RHS_TERMS = [[(0, 1), (3, 1)], [(0, 1)], [(1, 1), (3, -1)], [(2, 1), (0, -1)], [(3, 1)], [(0, 1), (1, 1)],
             [(2, 1), (3, 1)]]
INNER = [2, 4, 1, 3, 0, 5, 6]
OUTER = [4, 2, 1, 3, 0, 6, 5]
FIN = {2: (1, 4), 3: (2, 1), 6: (0, None), 5: (3, None)}
RIDE = {4: 1, 1: 2, 0: 0}
DOWN_OPS = ['s', 'a', 'u', 'v', 'd', 'us', 'vs']
DOWN_IN = [4, 2, 0, 6, 3, 1, 5]
DOWN_AT = {11: [4], 19: [1], 25: [2, 5], 27: [0, 3, 6]}


def _kernel(xt_hbm, c_hbm, wqkv_hbm, wo_hbm, w1_hbm, w3_hbm, w2t_hbm, wmod_hbm, out_hbm,
            x_v, c_v, wqkv_v, wo_v, wmod_v, w1_v, w3_v, w2t_v, tq_s, wt_s, wot_s, mod_s, gcol_s,
            part_s, q_s, kv_s, o_s, x1_s, a_s, acc_s, out_v, sems, xsems, osems):
    a_b, o_b, wt_b, wot_b = [r.bitcast(bf16) for r in (a_s, o_s, wt_s, wot_s)]

    def cp(src, dst, k):
        return pltpu.make_async_copy(src, dst, sems.at[k])

    def c_x(t):
        return pltpu.make_async_copy(xt_hbm.at[:, _ds(t * RB, RB)], x_v.at[t], xsems.at[t])

    c_c = cp(c_hbm, c_v, 0)
    c_ma = cp(wmod_hbm.at[:, 0:2 * D], wmod_v.at[:, 0:2 * D], 1)
    c_wq = [cp(wqkv_hbm.at[j * 128:min((j + 1) * 128, D), :], wqkv_v.at[j * 128:min((j + 1) * 128, D), :], 2 + j)
            for j in range(5)]
    c_wo = cp(wo_hbm, wo_v, 7)
    c_mb = cp(wmod_hbm.at[:, 2 * D:MB], wmod_v.at[:, 2 * D:MB], 8)
    c_mc = cp(wmod_hbm.at[:, MB:], wmod_v.at[:, MB:], 9)
    c_ffn = [cp(w1_hbm, w1_v, 10), cp(w3_hbm, w3_v, 11), cp(w2t_hbm, w2t_v, 12)]
    c_x(0).start(priority=0)
    for d in ([c_wq[0], c_c, c_ma] + c_wq[1:] + [c_wo, c_mb] + [c_x(t) for t in range(2, NBLK)]
              + [c_mc] + c_ffn):
        d.start(priority=1)

    def mod_cols(lo, hi):
        cc = c_v[...].astype(f32)
        sc = jnp.broadcast_to((cc * jax.nn.sigmoid(cc)).astype(bf16), (16, D))
        return _mm(sc, wmod_v[:, lo:hi])

    def col_bcast(row):
        return jnp.broadcast_to(row, (128, D)).T

    def modulate1(xn):
        return xn * (1.0 + mod_s[1, 0:1, :]) + mod_s[0, 0:1, :]

    def qkv_part(h1, lo, hi):
        return _mmt(h1[:, lo:hi].astype(bf16), wt_b[:, lo:hi])

    def store_qkv(qkv, par):
        rk = pl.ds(HALO, RB)
        lane = jax.lax.broadcasted_iota(jnp.int32, (RB, 128), 1)
        for j in range(4):
            q_s[par, j] = qkv[:, j * 128:(j + 1) * 128]
            kv_s[par, j, rk, :] = qkv[:, 512 + j * 128:512 + (j + 1) * 128]
            kv_s[par, 5 + j, rk, :] = qkv[:, 1024 + j * 128:1024 + (j + 1) * 128]
        t4 = qkv[:, 1536:1664]
        q_s[par, 4] = jnp.where(lane < 64, t4, 0.0)
        kv_s[par, 4, rk, :] = pltpu.roll(t4, 64, 1)
        kv_s[par, 9, rk, :] = qkv[:, 1664:1792]

    def s1(t, par):
        kv_s[par, :, 0:HALO, :] = kv_s[1 - par, :, RB:RB + HALO, :]
        h1 = modulate1(_ln_t(x_v[t].astype(f32)).T)
        tl = qkv_part(h1, KM, D)
        store_qkv(qkv_part(h1, 0, KM) + tl, par)

    def s2(par, first=False, skew=0):
        qscale = (DH ** -0.5) * LOG2E
        ngrp = RB // GR
        st = {}

        def kv(j, g, w):
            return kv_s[par, j, pl.ds(g * GR + HALO - DIL * w, GR), :]

        def scores(g):
            q = [q_s[par, j, g * GR:(g + 1) * GR, :] * qscale for j in range(5)]
            ps = []
            for w in range(W):
                p = q[0] * kv(0, g, w)
                for j in range(1, 5):
                    p = p + q[j] * kv(j, g, w)
                ps.append(p)
            p = jnp.concatenate(ps, axis=0)
            st[g] = (p, pltpu.roll(p, 64, 1))

        def fold(g):
            p, pr = st[g]
            p = p + pr
            st[g] = (p, pltpu.roll(p, 32, 1))

        def mix(g):
            p, pr = st.pop(g)
            p = p + pr
            lg = [p[w * GR:(w + 1) * GR] for w in range(W)]
            if first and g * GR < HALO:
                pos = g * GR + jax.lax.broadcasted_iota(jnp.int32, (GR, 128), 0)
                lg = [lg[0]] + [jnp.where(pos >= DIL * w, lg[w], -1e9 * LOG2E) for w in range(1, W)]
            m = jnp.maximum(jnp.maximum(jnp.maximum(lg[0], lg[1]), jnp.maximum(lg[2], lg[3])),
                            jnp.maximum(jnp.maximum(lg[4], lg[5]), jnp.maximum(lg[6], lg[7])))
            e = [jnp.exp2(l - m) for l in lg]
            den = ((e[0] + e[1]) + (e[2] + e[3])) + ((e[4] + e[5]) + (e[6] + e[7]))
            inv = pl.reciprocal(den, approx=True)
            inv = inv * (2.0 - den * inv)
            for j in range(5):
                a = e[0] * kv(5 + j, g, 0)
                for w in range(1, W):
                    a = a + e[w] * kv(5 + j, g, w)
                if g % 2 == 0:
                    st[('o', j)] = a * inv
                else:
                    both = jnp.concatenate([st.pop(('o', j)), a * inv], axis=0)
                    o_b[(g - 1) * GR:(g + 1) * GR, (par * 5 + j) * 128:(par * 5 + j + 1) * 128] = both.astype(bf16)

        for i in range(ngrp + 2 * skew):
            if i < ngrp:
                scores(i)
            if 0 <= i - skew < ngrp:
                fold(i - skew)
            if 0 <= i - 2 * skew < ngrp:
                mix(i - 2 * skew)

    def s3(t, par):
        att = _mmt(wot_b[...], o_b[:, par * 640:(par + 1) * 640])
        ga = jnp.concatenate([gcol_s[0]] * (RB // 128), axis=1)
        x1 = x_v[t].astype(f32) + ga * att
        x1_s[:, _ds(t * RB, RB)] = x1
        h = _ln_t(x1).T * (1.0 + mod_s[3, 0:1, :]) + mod_s[2, 0:1, :]
        rr = _ds(t * QB, QB)
        for ka, y in enumerate(_lhs7(_quads(h[:, 0:KM]))):
            for kb, z in enumerate(_lhs7(_quads(y))):
                a_b[rr, (ka * 7 + kb) * 128:(ka * 7 + kb + 1) * 128] = z.astype(bf16)
        for i in range(4):
            a_b[rr, (49 + i) * 128:(49 + i) * 128 + 64] = h[i * QB:(i + 1) * QB, KM:D].astype(bf16)

    def prep_wq(j):
        w = 128 if j < 4 else 64
        tq_s[j, 0:3 * D, 0:w] = wqkv_v[j * 128:j * 128 + w, :].astype(f32).T
        for sec in range(3):
            for d in range(DH):
                g = tq_s[j, pl.ds(sec * D + d, H, stride=DH), :]
                dst = _qkv_row(sec, d)
                wt_b[dst:dst + 32, j * 128:(j + 1) * 128] = g.astype(bf16)

    def prep_wo():
        for j in range(5):
            w = 128 if j < 4 else 64
            tq_s[j, 0:D, 0:w] = wo_v[:, j * 128:j * 128 + w].astype(f32)
        for j in range(5):
            w = 128 if j < 4 else 64
            parts = [tq_s[j, pl.ds(d, H, stride=DH), :] for d in range(DH)] + [jnp.zeros((64, 128), f32)]
            wot_b[j * 128:j * 128 + w, :] = jnp.concatenate(parts, axis=0).T[0:w, :].astype(bf16)

    def clear(k, carry):
        acc_s[k // 7, pl.ds((k % 7) * 7, 7)] = jnp.zeros((7, QD, 128), f32)
        return carry

    kv_s[0, :, 0:HALO, :] = jnp.zeros((10, HALO, 128), f32)
    wt_b[3 * D:NQ, :] = jnp.zeros((NQ - 3 * D, 640), bf16)
    tq_s[0:4, 3 * D:, :] = jnp.zeros((4, 24, 128), f32)
    tq_s[4] = jnp.zeros((3 * D + 24, 128), f32)
    a_b[:, 49 * 128:] = jnp.zeros((QS, 4 * 128), bf16)
    o_b[:, 640 + KM:] = jnp.zeros((RB, 128), bf16)
    jax.lax.fori_loop(0, Z0, clear, 0)
    c_x(0).wait()
    c_wq[0].wait()
    xn = _ln_t(x_v[0].astype(f32)).T
    prep_wq(0)
    jax.lax.fori_loop(Z0, Z1, clear, 0)
    c_c.wait()
    c_ma.wait()
    mod = mod_cols(0, 2 * D)
    mod_s[0] = mod[0:8, 0:D]
    mod_s[1] = mod[0:8, D:2 * D]
    h1 = modulate1(xn)
    c_wq[1].wait()
    c_x(1).start(priority=0)
    part_s[...] = qkv_part(h1, 0, 128)
    prep_wq(1)
    c_wq[2].wait()
    part_s[...] += qkv_part(h1, 128, 256)
    prep_wq(2)
    c_wq[3].wait()
    c_wq[4].wait()
    c_x(1).wait()
    part = part_s[...] + qkv_part(h1, 256, 384)
    prep_wq(3)
    prep_wq(4)
    store_qkv(part + qkv_part(h1, 384, D), 0)
    o_b[:, 640:640 + D] = modulate1(_ln_t(x_v[1].astype(f32)).T).astype(bf16)

    c_wo.wait()
    prep_wo()
    kv_s[1, :, 0:HALO, :] = kv_s[0, :, RB:RB + HALO, :]
    tl = _mmt(o_b[:, 640 + KM:640 + D], wt_b[:, KM:D])
    store_qkv(_mmt(o_b[:, 640:640 + KM], wt_b[:, 0:KM]) + tl, 1)
    s2(0, first=True, skew=1)
    c_mb.wait()
    mod = mod_cols(2 * D, MB)
    gcol_s[0] = col_bcast(mod[0:1, 0:D])
    mod_s[2] = mod[0:8, D:2 * D]
    mod_s[3] = mod[0:8, 2 * D:3 * D]
    acc_s[3, (Z1 - 21) * 7:49] = jnp.zeros(((28 - Z1) * 7, QD, 128), f32)

    def a_step(t, par):
        s3(t - 2, par)
        s1(t, par)
        s2(1 - par)

    def a_body(t, carry):
        c_x(t).wait()
        for par in range(2):
            pl.when(t % 2 == par)(functools.partial(a_step, t, par))
        return carry

    jax.lax.fori_loop(2, NBLK, a_body, 0)

    c_mc.wait()
    gcol_s[1] = col_bcast(mod_cols(MB - 128, 6 * D)[0:1, 64:64 + D])
    s3(NBLK - 2, 0)
    s2(1)
    s3(NBLK - 1, 1)
    for d in c_ffn:
        d.wait()

    def b_body(ci, carry):
        n = _ds(ci * FC, FC)
        w_out = [_rhs7(_quads(w[0:KM, n].astype(f32))) for w in (w1_v, w3_v)]
        w_tail = [w[KM:D, n] for w in (w1_v, w3_v)]
        w2_out = _lhs7(_quads(w2t_v[:, n].astype(f32)))
        early, mo, gate, psum = [{}, {}], [[None] * 7, [None] * 7], {}, [{}, {}]
        hid, hblk = {}, {}

        def tail(x, oq, iq):
            i, j = (oq // 2) * 2 + iq // 2, (oq % 2) * 2 + iq % 2
            return _mm(a_b[:, (49 + i) * 128:(49 + i) * 128 + 64], w_tail[x][:, j * 128:(j + 1) * 128])

        def chain(x, v, terms, iq):
            for k, sg in terms:
                v = v + mo[x][k][iq] if (sg > 0) != (iq == 1) else v - mo[x][k][iq]
            return v

        def final(x, a, iq):
            if a == 0:
                m1 = mo[x][0][iq] if iq != 1 else -mo[x][0][iq]
                psum[x][(0, iq)] = chain(x, m1, [(3, 1), (4, -1)], iq)
                psum[x][(3, iq)] = chain(x, m1, [(2, 1), (1, -1)], iq)
            if a not in FIN:
                return
            oq, partner = FIN[a]
            v = chain(x, early[x][oq] if iq == 1 else tail(x, oq, iq), [(a, 1)], iq)
            v = v + psum[x][(oq, iq)] if partner is None else chain(x, v, [(partner, 1)], iq)
            if x == 0:
                gate[(oq, iq)] = v
                return
            hv = _swiglu(gate[(oq, iq)], v)
            if oq == 1:
                hid[('d', iq)] = hv
            elif oq == 2:
                hid[('a', iq)] = hv
                hid[('s', iq)] = hv + hid[('d', iq)]
            elif oq == 0:
                hid[('u', iq)] = hv - hid[('d', iq)]
            else:
                hid[('v', iq)] = hv - hid[('a', iq)]

        def hidden(oq, j):
            if (oq, j) not in hblk:
                kk, nn = divmod(j, 2)
                parts = []
                for t in range(4):
                    rs = slice((2 * t + nn) * QB, (2 * t + nn + 1) * QB)
                    parts += [hid[(oq, kk)][rs], hid[(oq, 2 + kk)][rs]]
                hblk[(oq, j)] = jnp.concatenate(parts, axis=0)
            return hblk[(oq, j)]

        def down(wave):
            for a in DOWN_AT.get(wave, []):
                lhs = [z.astype(bf16) for z in _lhs7(_quads(w2_out[a]))]
                for b in DOWN_IN:
                    terms = [(hidden(i, j), sj) for i in DOWN_OPS[a] for j, sj in RHS_TERMS[b]]
                    if len(terms) == 4:
                        terms = [terms[0], terms[3], terms[1], terms[2]]
                    r = _mmt(lhs[b], _lin(terms).astype(bf16))
                    for t in range(4):
                        acc_s[t, a * 7 + b] += r[:, t * 128:(t + 1) * 128]

        wave = 0
        for a in OUTER:
            if a == 5:
                for x in range(2):
                    early[x][3] = tail(x, 3, 1)
            for x in range(2):
                rhs = [z.astype(bf16) for z in _rhs7n(_quads(w_out[x][a]))]
                m = [None] * 7
                for b in INNER[:4]:
                    m[b] = _mm(a_b[:, (a * 7 + b) * 128:(a * 7 + b + 1) * 128], rhs[b])
                sa = [m[3] + m[4], m[2] + m[4], m[1] + m[3], m[2] + m[1]]
                mo[x][a] = [None, sa[1], sa[2], None]
                final(x, a, 1)
                final(x, a, 2)
                down(wave)
                for b in INNER[4:]:
                    m[b] = _mm(a_b[:, (a * 7 + b) * 128:(a * 7 + b + 1) * 128], rhs[b])
                if a in RIDE:
                    early[x][RIDE[a]] = tail(x, RIDE[a], 1)
                mo[x][a] = [(m[0] + m[6]) + sa[0], sa[1], sa[2], (m[0] + m[5]) - sa[3]]
                if a not in (2, 3):
                    final(x, a, 0)
                    final(x, a, 3)
                elif x == 1:
                    for iq in (0, 3):
                        final(0, a, iq)
                        final(1, a, iq)
                down(wave + 1)
                wave += 2
        return carry

    jax.lax.fori_loop(0, F // FC, b_body, 0)

    copies = []
    r0 = 0
    for ck, rows in enumerate(ECH):
        for r in range(r0, r0 + rows, ER):
            for t in range(4):
                cs = slice(t * QS, (t + 1) * QS)
                mo = [_out4([acc_s[t, a * 7 + b, r:r + ER, :] for b in range(7)]) for a in range(7)]
                cq = [_out4([mo[a][i] for a in range(7)]) for i in range(4)]
                for mq in range(4):
                    rs = slice(mq * QD + r, mq * QD + r + ER)
                    row = jnp.concatenate([cq[(mq % 2) * 2 + nn][(mq // 2) * 2 + 1 - hh]
                                           for nn in range(2) for hh in range(2)], axis=1)
                    gb = jnp.concatenate([gcol_s[1, rs, :]] * 4, axis=1)
                    out_v[rs, cs] = (x1_s[rs, cs] + gb * row).astype(bf16)
        for mq in range(4):
            rs = slice(mq * QD + r0, mq * QD + r0 + rows)
            d = pltpu.make_async_copy(out_v.at[rs, :], out_hbm.at[rs, :], osems.at[ck * 4 + mq])
            d.start()
            copies.append(d)
        r0 += rows
    for d in copies:
        d.wait()


@jax.jit
def pallas_adaLN_cond__sliding_local_dilated__glu_gated_swiglu__prompt_kernel(
    A_x: jax.Array,
    A_wqkv: jax.Array,
    A_wo: jax.Array,
    B_x: jax.Array,
    B_w1: jax.Array,
    B_w3: jax.Array,
    B_w2: jax.Array,
    c: jax.Array,
    w_mod: jax.Array,
):
    del B_x
    hbm = pl.BlockSpec(memory_space=pl.ANY)
    out_t = pl.pallas_call(
        _kernel,
        in_specs=[hbm] * 8,
        out_specs=hbm,
        out_shape=jax.ShapeDtypeStruct((D, S), bf16),
        scratch_shapes=[
            pltpu.VMEM((NBLK, D, RB), bf16),
            pltpu.VMEM((1, D), bf16),
            pltpu.VMEM((D, 3 * D), bf16),
            pltpu.VMEM((D, D), bf16),
            pltpu.VMEM((D, 6 * D), bf16),
            pltpu.VMEM((D, F), bf16),
            pltpu.VMEM((D, F), bf16),
            pltpu.VMEM((D, F), bf16),
            pltpu.VMEM((5, 3 * D + 24, 128), f32),
            pltpu.VMEM((NQ // 2, 640), u32),
            pltpu.VMEM((D // 2, 640), u32),
            pltpu.VMEM((4, 8, D), f32),
            pltpu.VMEM((2, D, 128), f32),
            pltpu.VMEM((RB, NQ), f32),
            pltpu.VMEM((2, 5, RB, 128), f32),
            pltpu.VMEM((2, 10, RB + HALO, 128), f32),
            pltpu.VMEM((RB // 2, 2 * 640), u32),
            pltpu.VMEM((D, S), f32),
            pltpu.VMEM((QS // 2, 53 * 128), u32),
            pltpu.VMEM((4, 49, QD, 128), f32),
            pltpu.VMEM((D, S), bf16),
            pltpu.SemaphoreType.DMA((13,)),
            pltpu.SemaphoreType.DMA((NBLK,)),
            pltpu.SemaphoreType.DMA((4 * len(ECH),)),
        ],
        compiler_params=pltpu.CompilerParams(vmem_limit_bytes=110 * 1024 * 1024),
        name="adaln_blk",
    )(A_x[0].T, c, A_wqkv, A_wo, B_w1, B_w3, B_w2.T, w_mod)
    return out_t.T[None]
```

```python
import functools

import jax
import jax.numpy as jnp
import jax.experimental.pallas as pl
import jax.experimental.pallas.tpu as pltpu

S, D, F = 2048, 576, 4608
H, DH, W, DIL = 32, 18, 8, 2
EPS = 1e-5
LOG2E = 1.4426950408889634
f32, bf16, u32 = jnp.float32, jnp.bfloat16, jnp.uint32

HALO = 16
RB = 256
NBLK = S // RB
GR = 8
NQ = 1792
KM = 512
FC = 512
QD, QS, QB = D // 4, S // 4, RB // 4
MB = 23 * 128
ER = 16
ECH = (16, 32, 48, 48)
Z0, Z1 = 13, 23


def _mm(a, b):
    return jnp.dot(a, b, preferred_element_type=f32)


def _mmt(a, b):
    return jax.lax.dot_general(a, b, (((1,), (1,)), ((), ())), preferred_element_type=f32)


def _ln_t(xt):
    m = jnp.sum(xt, axis=0, keepdims=True) * (1.0 / D)
    xm = m - xt
    v = jnp.sum(xm * xm, axis=0, keepdims=True) * (1.0 / D)
    return (xt - m) * jax.lax.rsqrt(v + EPS)


def _ln_t_shifted(xt):
    piv = xt[0:1, :]
    d = xt - piv
    md = jnp.sum(d, axis=0, keepdims=True) * (1.0 / D)
    m2 = jnp.sum(d * d, axis=0, keepdims=True) * (1.0 / D)
    v = jnp.maximum(m2 - md * md, 0.0)
    return (xt - (piv + md)) * jax.lax.rsqrt(v + EPS)


def _swiglu(g, u):
    t = 0.5 * g
    tu = t * u
    return tu + tu * jnp.tanh(t)


def _ds(start, size):
    if isinstance(start, int):
        return pl.ds(start, size)
    return pl.ds(pl.multiple_of(start, size), size)


def _qkv_row(sec, d):
    return sec * 512 + d * 32 if d < 16 else 1536 + sec * 64 + (d - 16) * 32


def _quads(x):
    m, n = x.shape[0] // 2, x.shape[1] // 2
    return [x[:m, :n], x[:m, n:], x[m:, :n], x[m:, n:]]


def _lhs7(x):
    a, b, c, d = x
    return [a + d, c + d, a, d, a + b, c - a, b - d]


def _rhs7(x):
    a, b, c, d = x
    return [a + d, a, b - d, c - a, d, a + b, c + d]


def _rhs7n(x):
    a, b, c, d = x
    return [a + d, a, d - b, c - a, -d, a + b, c + d]


def _out4(m):
    m1, m2, m3, m4, m5, m6, m7 = m
    return [(m1 + m7) + (m4 - m5), m3 + m5, m2 + m4, (m1 + m6) + (m3 - m2)]


def _lin(terms):
    v = None
    for t, sg in terms:
        v = t if v is None else (v + t if sg > 0 else v - t)
    return v


RHS_TERMS = [[(0, 1), (3, 1)], [(0, 1)], [(1, 1), (3, -1)], [(2, 1), (0, -1)], [(3, 1)], [(0, 1), (1, 1)],
             [(2, 1), (3, 1)]]
INNER = [2, 4, 1, 3, 0, 5, 6]
OUTER = [4, 2, 1, 3, 0, 6, 5]
FIN = {2: (1, 4), 3: (2, 1), 6: (0, None), 5: (3, None)}
RIDE = {4: 1, 1: 2, 0: 0}
DOWN_OPS = ['s', 'a', 'u', 'v', 'd', 'us', 'vs']
DOWN_IN = [4, 2, 0, 6, 3, 1, 5]
DOWN_AT = {11: [4], 19: [1], 25: [2, 5], 27: [0, 3, 6]}


def _kernel(xt_hbm, c_hbm, wqkv_hbm, wo_hbm, w1_hbm, w3_hbm, w2t_hbm, wmod_hbm, out_hbm,
            x_v, c_v, wqkv_v, wo_v, wmod_v, w1_v, w3_v, w2t_v, tq_s, wt_s, wot_s, mod_s, gcol_s,
            part_s, q_s, kv_s, o_s, x1_s, a_s, acc_s, out_v, sems, xsems, osems):
    a_b, o_b, wt_b, wot_b = [r.bitcast(bf16) for r in (a_s, o_s, wt_s, wot_s)]

    def cp(src, dst, k):
        return pltpu.make_async_copy(src, dst, sems.at[k])

    def c_x(t):
        return pltpu.make_async_copy(xt_hbm.at[:, _ds(t * RB, RB)], x_v.at[t], xsems.at[t])

    c_c = cp(c_hbm, c_v, 0)
    c_ma = cp(wmod_hbm.at[:, 0:2 * D], wmod_v.at[:, 0:2 * D], 1)
    c_wq = [cp(wqkv_hbm.at[j * 128:min((j + 1) * 128, D), :], wqkv_v.at[j * 128:min((j + 1) * 128, D), :], 2 + j)
            for j in range(5)]
    c_wo = cp(wo_hbm, wo_v, 7)
    c_mb = cp(wmod_hbm.at[:, 2 * D:MB], wmod_v.at[:, 2 * D:MB], 8)
    c_mc = cp(wmod_hbm.at[:, MB:], wmod_v.at[:, MB:], 9)
    c_ffn = [cp(w1_hbm, w1_v, 10), cp(w3_hbm, w3_v, 11), cp(w2t_hbm, w2t_v, 12)]
    c_x(0).start(priority=0)
    for d in ([c_wq[0], c_c, c_ma] + c_wq[1:] + [c_wo, c_mb] + [c_x(t) for t in range(2, NBLK)]
              + [c_mc] + c_ffn):
        d.start(priority=1)

    def mod_cols(lo, hi):
        cc = c_v[...].astype(f32)
        sc = jnp.broadcast_to((cc * jax.nn.sigmoid(cc)).astype(bf16), (16, D))
        return _mm(sc, wmod_v[:, lo:hi])

    def col_bcast(row):
        return jnp.broadcast_to(row, (128, D)).T

    def modulate1(xn):
        return xn * (1.0 + mod_s[1, 0:1, :]) + mod_s[0, 0:1, :]

    def qkv_part(h1, lo, hi):
        return _mmt(h1[:, lo:hi].astype(bf16), wt_b[:, lo:hi])

    def store_qkv(qkv, par):
        rk = pl.ds(HALO, RB)
        lane = jax.lax.broadcasted_iota(jnp.int32, (RB, 128), 1)
        for j in range(4):
            q_s[par, j] = qkv[:, j * 128:(j + 1) * 128]
            kv_s[par, j, rk, :] = qkv[:, 512 + j * 128:512 + (j + 1) * 128]
            kv_s[par, 5 + j, rk, :] = qkv[:, 1024 + j * 128:1024 + (j + 1) * 128]
        t4 = qkv[:, 1536:1664]
        q_s[par, 4] = jnp.where(lane < 64, t4, 0.0)
        kv_s[par, 4, rk, :] = pltpu.roll(t4, 64, 1)
        kv_s[par, 9, rk, :] = qkv[:, 1664:1792]

    def s1(t, par):
        kv_s[par, :, 0:HALO, :] = kv_s[1 - par, :, RB:RB + HALO, :]
        h1 = modulate1(_ln_t(x_v[t].astype(f32)).T)
        tl = qkv_part(h1, KM, D)
        store_qkv(qkv_part(h1, 0, KM) + tl, par)

    def s2(par, first=False, skew=0):
        qscale = (DH ** -0.5) * LOG2E
        ngrp = RB // GR
        st = {}

        def kv(j, g, w):
            return kv_s[par, j, pl.ds(g * GR + HALO - DIL * w, GR), :]

        def scores(g):
            q = [q_s[par, j, g * GR:(g + 1) * GR, :] * qscale for j in range(5)]
            ps = []
            for w in range(W):
                p = q[4] * kv(4, g, w)
                for j in (3, 2, 1, 0):
                    p = p + q[j] * kv(j, g, w)
                ps.append(p)
            p = jnp.concatenate(ps, axis=0)
            st[g] = (p, pltpu.roll(p, 64, 1))

        def fold(g):
            p, pr = st[g]
            p = p + pr
            st[g] = (p, pltpu.roll(p, 32, 1))

        def mix(g):
            p, pr = st.pop(g)
            p = p + pr
            lg = [p[w * GR:(w + 1) * GR] for w in range(W)]
            if first and g * GR < HALO:
                pos = g * GR + jax.lax.broadcasted_iota(jnp.int32, (GR, 128), 0)
                lg = [lg[0]] + [jnp.where(pos >= DIL * w, lg[w], -1e9 * LOG2E) for w in range(1, W)]
            m = jnp.maximum(jnp.maximum(jnp.maximum(lg[0], lg[1]), jnp.maximum(lg[2], lg[3])),
                            jnp.maximum(jnp.maximum(lg[4], lg[5]), jnp.maximum(lg[6], lg[7])))
            e = [jnp.exp2(l - m) for l in lg]
            den = ((e[0] + e[1]) + (e[2] + e[3])) + ((e[4] + e[5]) + (e[6] + e[7]))
            inv = pl.reciprocal(den, approx=True)
            inv = inv * (2.0 - den * inv)
            for j in range(5):
                a = e[0] * kv(5 + j, g, 0)
                for w in range(1, W):
                    a = a + e[w] * kv(5 + j, g, w)
                if g % 2 == 0:
                    st[('o', j)] = a * inv
                else:
                    both = jnp.concatenate([st.pop(('o', j)), a * inv], axis=0)
                    o_b[(g - 1) * GR:(g + 1) * GR, (par * 5 + j) * 128:(par * 5 + j + 1) * 128] = both.astype(bf16)

        for i in range(ngrp + 2 * skew):
            if i < ngrp:
                scores(i)
            if 0 <= i - skew < ngrp:
                fold(i - skew)
            if 0 <= i - 2 * skew < ngrp:
                mix(i - 2 * skew)

    def s3(t, par):
        att = _mmt(wot_b[...], o_b[:, par * 640:(par + 1) * 640])
        ga = jnp.concatenate([gcol_s[0]] * (RB // 128), axis=1)
        x1 = x_v[t].astype(f32) + ga * att
        x1_s[:, _ds(t * RB, RB)] = x1
        h = _ln_t_shifted(x1).T * (1.0 + mod_s[3, 0:1, :]) + mod_s[2, 0:1, :]
        rr = _ds(t * QB, QB)
        for ka, y in enumerate(_lhs7(_quads(h[:, 0:KM]))):
            for kb, z in enumerate(_lhs7(_quads(y))):
                a_b[rr, (ka * 7 + kb) * 128:(ka * 7 + kb + 1) * 128] = z.astype(bf16)
        for i in range(4):
            a_b[rr, (49 + i) * 128:(49 + i) * 128 + 64] = h[i * QB:(i + 1) * QB, KM:D].astype(bf16)

    def prep_wq(j):
        w = 128 if j < 4 else 64
        tq_s[j, 0:3 * D, 0:w] = wqkv_v[j * 128:j * 128 + w, :].astype(f32).T
        for sec in range(3):
            for d in range(DH):
                g = tq_s[j, pl.ds(sec * D + d, H, stride=DH), :]
                dst = _qkv_row(sec, d)
                wt_b[dst:dst + 32, j * 128:(j + 1) * 128] = g.astype(bf16)

    def prep_wo():
        for j in range(5):
            w = 128 if j < 4 else 64
            tq_s[j, 0:D, 0:w] = wo_v[:, j * 128:j * 128 + w].astype(f32)
        for j in range(5):
            w = 128 if j < 4 else 64
            parts = [tq_s[j, pl.ds(d, H, stride=DH), :] for d in range(DH)] + [jnp.zeros((64, 128), f32)]
            wot_b[j * 128:j * 128 + w, :] = jnp.concatenate(parts, axis=0).T[0:w, :].astype(bf16)

    def clear(k, carry):
        acc_s[k // 7, pl.ds((k % 7) * 7, 7)] = jnp.zeros((7, QD, 128), f32)
        return carry

    kv_s[0, :, 0:HALO, :] = jnp.zeros((10, HALO, 128), f32)
    wt_b[3 * D:NQ, :] = jnp.zeros((NQ - 3 * D, 640), bf16)
    tq_s[0:4, 3 * D:, :] = jnp.zeros((4, 24, 128), f32)
    tq_s[4] = jnp.zeros((3 * D + 24, 128), f32)
    a_b[:, 49 * 128:] = jnp.zeros((QS, 4 * 128), bf16)
    o_b[:, 640 + KM:] = jnp.zeros((RB, 128), bf16)
    jax.lax.fori_loop(0, Z0, clear, 0)
    c_x(0).wait()
    c_wq[0].wait()
    xn = _ln_t(x_v[0].astype(f32)).T
    prep_wq(0)
    jax.lax.fori_loop(Z0, Z1, clear, 0)
    c_c.wait()
    c_ma.wait()
    mod = mod_cols(0, 2 * D)
    mod_s[0] = mod[0:8, 0:D]
    mod_s[1] = mod[0:8, D:2 * D]
    h1 = modulate1(xn)
    c_wq[1].wait()
    c_x(1).start(priority=0)
    part_s[...] = qkv_part(h1, 0, 128)
    prep_wq(1)
    c_wq[2].wait()
    part_s[...] += qkv_part(h1, 128, 256)
    prep_wq(2)
    c_wq[3].wait()
    c_wq[4].wait()
    c_x(1).wait()
    part = part_s[...] + qkv_part(h1, 256, 384)
    prep_wq(3)
    prep_wq(4)
    store_qkv(part + qkv_part(h1, 384, D), 0)
    o_b[:, 640:640 + D] = modulate1(_ln_t(x_v[1].astype(f32)).T).astype(bf16)

    c_wo.wait()
    prep_wo()
    kv_s[1, :, 0:HALO, :] = kv_s[0, :, RB:RB + HALO, :]
    tl = _mmt(o_b[:, 640 + KM:640 + D], wt_b[:, KM:D])
    store_qkv(_mmt(o_b[:, 640:640 + KM], wt_b[:, 0:KM]) + tl, 1)
    s2(0, first=True, skew=1)
    c_mb.wait()
    mod = mod_cols(2 * D, MB)
    gcol_s[0] = col_bcast(mod[0:1, 0:D])
    mod_s[2] = mod[0:8, D:2 * D]
    mod_s[3] = mod[0:8, 2 * D:3 * D]
    acc_s[3, (Z1 - 21) * 7:49] = jnp.zeros(((28 - Z1) * 7, QD, 128), f32)

    def a_step(t, par):
        s3(t - 2, par)
        s1(t, par)
        s2(1 - par)

    def a_body(t, carry):
        c_x(t).wait()
        for par in range(2):
            pl.when(t % 2 == par)(functools.partial(a_step, t, par))
        return carry

    jax.lax.fori_loop(2, NBLK, a_body, 0)

    c_mc.wait()
    gcol_s[1] = col_bcast(mod_cols(MB - 128, 6 * D)[0:1, 64:64 + D])
    s3(NBLK - 2, 0)
    s2(1)
    s3(NBLK - 1, 1)
    for d in c_ffn:
        d.wait()

    def b_body(ci, carry):
        n = _ds(ci * FC, FC)
        w_out = [_rhs7(_quads(w[0:KM, n].astype(f32))) for w in (w1_v, w3_v)]
        w_tail = [w[KM:D, n] for w in (w1_v, w3_v)]
        w2_out = _lhs7(_quads(w2t_v[:, n].astype(f32)))
        early, mo, gate, psum = [{}, {}], [[None] * 7, [None] * 7], {}, [{}, {}]
        hid, hblk = {}, {}

        def tail(x, oq, iq):
            i, j = (oq // 2) * 2 + iq // 2, (oq % 2) * 2 + iq % 2
            return _mm(a_b[:, (49 + i) * 128:(49 + i) * 128 + 64], w_tail[x][:, j * 128:(j + 1) * 128])

        def chain(x, v, terms, iq):
            for k, sg in terms:
                v = v + mo[x][k][iq] if (sg > 0) != (iq == 1) else v - mo[x][k][iq]
            return v

        def final(x, a, iq):
            if a == 0:
                m1 = mo[x][0][iq] if iq != 1 else -mo[x][0][iq]
                psum[x][(0, iq)] = chain(x, m1, [(3, 1), (4, -1)], iq)
                psum[x][(3, iq)] = chain(x, m1, [(2, 1), (1, -1)], iq)
            if a not in FIN:
                return
            oq, partner = FIN[a]
            v = chain(x, early[x][oq] if iq == 1 else tail(x, oq, iq), [(a, 1)], iq)
            v = v + psum[x][(oq, iq)] if partner is None else chain(x, v, [(partner, 1)], iq)
            if x == 0:
                gate[(oq, iq)] = v
                return
            hv = _swiglu(gate[(oq, iq)], v)
            if oq == 1:
                hid[('d', iq)] = hv
            elif oq == 2:
                hid[('a', iq)] = hv
                hid[('s', iq)] = hv + hid[('d', iq)]
            elif oq == 0:
                hid[('u', iq)] = hv - hid[('d', iq)]
            else:
                hid[('v', iq)] = hv - hid[('a', iq)]

        def hidden(oq, j):
            if (oq, j) not in hblk:
                kk, nn = divmod(j, 2)
                parts = []
                for t in range(4):
                    rs = slice((2 * t + nn) * QB, (2 * t + nn + 1) * QB)
                    parts += [hid[(oq, kk)][rs], hid[(oq, 2 + kk)][rs]]
                hblk[(oq, j)] = jnp.concatenate(parts, axis=0)
            return hblk[(oq, j)]

        def down(wave):
            for a in DOWN_AT.get(wave, []):
                lhs = [z.astype(bf16) for z in _lhs7(_quads(w2_out[a]))]
                for b in DOWN_IN:
                    terms = [(hidden(i, j), sj) for i in DOWN_OPS[a] for j, sj in RHS_TERMS[b]]
                    if len(terms) == 4:
                        terms = [terms[0], terms[3], terms[1], terms[2]]
                    r = _mmt(lhs[b], _lin(terms).astype(bf16))
                    for t in range(4):
                        acc_s[t, a * 7 + b] += r[:, t * 128:(t + 1) * 128]

        wave = 0
        for a in OUTER:
            if a == 5:
                for x in range(2):
                    early[x][3] = tail(x, 3, 1)
            for x in range(2):
                rhs = [z.astype(bf16) for z in _rhs7n(_quads(w_out[x][a]))]
                m = [None] * 7
                for b in INNER[:4]:
                    m[b] = _mm(a_b[:, (a * 7 + b) * 128:(a * 7 + b + 1) * 128], rhs[b])
                sa = [m[3] + m[4], m[2] + m[4], m[1] + m[3], m[2] + m[1]]
                mo[x][a] = [None, sa[1], sa[2], None]
                final(x, a, 1)
                final(x, a, 2)
                down(wave)
                for b in INNER[4:]:
                    m[b] = _mm(a_b[:, (a * 7 + b) * 128:(a * 7 + b + 1) * 128], rhs[b])
                if a in RIDE:
                    early[x][RIDE[a]] = tail(x, RIDE[a], 1)
                mo[x][a] = [(m[0] + m[6]) + sa[0], sa[1], sa[2], (m[0] + m[5]) - sa[3]]
                if a not in (2, 3):
                    final(x, a, 0)
                    final(x, a, 3)
                elif x == 1:
                    for iq in (0, 3):
                        final(0, a, iq)
                        final(1, a, iq)
                down(wave + 1)
                wave += 2
        return carry

    jax.lax.fori_loop(0, F // FC, b_body, 0)

    copies = []
    r0 = 0
    for ck, rows in enumerate(ECH):
        for r in range(r0, r0 + rows, ER):
            for t in range(4):
                cs = slice(t * QS, (t + 1) * QS)
                mo = [_out4([acc_s[t, a * 7 + b, r:r + ER, :] for b in range(7)]) for a in range(7)]
                cq = [_out4([mo[a][i] for a in range(7)]) for i in range(4)]
                for mq in range(4):
                    rs = slice(mq * QD + r, mq * QD + r + ER)
                    row = jnp.concatenate([cq[(mq % 2) * 2 + nn][(mq // 2) * 2 + 1 - hh]
                                           for nn in range(2) for hh in range(2)], axis=1)
                    gb = jnp.concatenate([gcol_s[1, rs, :]] * 4, axis=1)
                    out_v[rs, cs] = (x1_s[rs, cs] + gb * row).astype(bf16)
        for mq in range(4):
            rs = slice(mq * QD + r0, mq * QD + r0 + rows)
            d = pltpu.make_async_copy(out_v.at[rs, :], out_hbm.at[rs, :], osems.at[ck * 4 + mq])
            d.start()
            copies.append(d)
        r0 += rows
    for d in copies:
        d.wait()


@jax.jit
def pallas_adaLN_cond__sliding_local_dilated__glu_gated_swiglu__prompt_kernel(
    A_x: jax.Array,
    A_wqkv: jax.Array,
    A_wo: jax.Array,
    B_x: jax.Array,
    B_w1: jax.Array,
    B_w3: jax.Array,
    B_w2: jax.Array,
    c: jax.Array,
    w_mod: jax.Array,
):
    del B_x
    hbm = pl.BlockSpec(memory_space=pl.ANY)
    out_t = pl.pallas_call(
        _kernel,
        in_specs=[hbm] * 8,
        out_specs=hbm,
        out_shape=jax.ShapeDtypeStruct((D, S), bf16),
        scratch_shapes=[
            pltpu.VMEM((NBLK, D, RB), bf16),
            pltpu.VMEM((1, D), bf16),
            pltpu.VMEM((D, 3 * D), bf16),
            pltpu.VMEM((D, D), bf16),
            pltpu.VMEM((D, 6 * D), bf16),
            pltpu.VMEM((D, F), bf16),
            pltpu.VMEM((D, F), bf16),
            pltpu.VMEM((D, F), bf16),
            pltpu.VMEM((5, 3 * D + 24, 128), f32),
            pltpu.VMEM((NQ // 2, 640), u32),
            pltpu.VMEM((D // 2, 640), u32),
            pltpu.VMEM((4, 8, D), f32),
            pltpu.VMEM((2, D, 128), f32),
            pltpu.VMEM((RB, NQ), f32),
            pltpu.VMEM((2, 5, RB, 128), f32),
            pltpu.VMEM((2, 10, RB + HALO, 128), f32),
            pltpu.VMEM((RB // 2, 2 * 640), u32),
            pltpu.VMEM((D, S), f32),
            pltpu.VMEM((QS // 2, 53 * 128), u32),
            pltpu.VMEM((4, 49, QD, 128), f32),
            pltpu.VMEM((D, S), bf16),
            pltpu.SemaphoreType.DMA((13,)),
            pltpu.SemaphoreType.DMA((NBLK,)),
            pltpu.SemaphoreType.DMA((4 * len(ECH),)),
        ],
        compiler_params=pltpu.CompilerParams(vmem_limit_bytes=110 * 1024 * 1024),
        name="adaln_blk",
    )(A_x[0].T, c, A_wqkv, A_wo, B_w1, B_w3, B_w2.T, w_mod)
    return out_t.T[None]
```
